```python
import jax
import jax.numpy as jnp

def _softmax(x, axis=-1):
    return jax.nn.softmax(x, axis=axis)

def _gelu(x):
    return jax.nn.gelu(x, approximate=True)

def _silu(x):
    return jax.nn.silu(x)

def _sigmoid(x):
    return jax.nn.sigmoid(x)

def _layernorm(x, axis=-1, eps=1e-05):
    m = jnp.mean(x, axis=axis, keepdims=True)
    v = jnp.var(x, axis=axis, keepdims=True)
    return (x - m) / jnp.sqrt(v + eps)

def _scatter_add(tgt, idx, src, axis=0):
    return tgt.at[idx].add(src)

def _segment_sum(src, seg, n):
    return jax.ops.segment_sum(src, seg, n)

class _Rng:

    def __init__(self, key):
        self._k = key

    def _next(self):
        self._k, sub = jax.random.split(self._k)
        return sub

    def normal(self, shape):
        return jax.random.normal(self._next(), shape, dtype=jnp.bfloat16)

    def randint(self, lo, hi, shape):
        return jax.random.randint(self._next(), shape, lo, hi, dtype=jnp.int32)

    def uniform(self, shape, lo=0.0, hi=1.0):
        return jax.random.uniform(self._next(), shape, jnp.bfloat16, lo, hi)

    def permutation(self, n):
        return jax.random.permutation(self._next(), n)
kernel_name = 'adaLN_cond__sliding_block_cached__mixer_channel_mlp__decode'

def setup_inputs():
    _rng = _Rng(jax.random.key(int.from_bytes(__import__("os").urandom(4), "little")))
    _w = lambda a: (lambda t: t.astype(jnp.bfloat16) if jnp.issubdtype(t.dtype, jnp.floating) else t)(jnp.asarray(a))

    def _A_setup():
        B, Sq, D = (8, 1, 640)
        Hq, Hkv, Sk, Dh = (32, 32, 4096, 192)
        assert Hq % Hkv == 0, (Hq, Hkv)
        return {'x': _w((lambda *s: _rng.normal(s) * 0.05)(B, Sq, D)), 'k_cache': _w((lambda *s: _rng.normal(s) * 0.05)(B, Hkv, Sk, Dh)), 'v_cache': _w((lambda *s: _rng.normal(s) * 0.05)(B, Hkv, Sk, Dh)), 'wq': _w((lambda *s: _rng.normal(s) * 0.05)(D, Hq * Dh) * D ** (-0.5)), 'wo': _w((lambda *s: _rng.normal(s) * 0.05)(Hq * Dh, D) * (Hq * Dh) ** (-0.5))}
    _A_in = _A_setup()

    def _B_setup():
        B, S, D, F = (8, 1, 640, 1536)
        return {'x': _w((lambda *s: _rng.normal(s) * 0.05)(B, S, D)), 'w1': _w((lambda *s: _rng.normal(s) * 0.05)(D, F) * D ** (-0.5)), 'b1': _w((lambda *s: _rng.normal(s) * 0.05)(F)), 'w2': _w((lambda *s: _rng.normal(s) * 0.05)(F, D) * F ** (-0.5)), 'b2': _w((lambda *s: _rng.normal(s) * 0.05)(D))}
    _B_in = _B_setup()
    return {'A_x': _A_in['x'], 'A_k_cache': _A_in['k_cache'], 'A_v_cache': _A_in['v_cache'], 'A_wq': _A_in['wq'], 'A_wo': _A_in['wo'], 'B_x': _B_in['x'], 'B_w1': _B_in['w1'], 'B_b1': _B_in['b1'], 'B_w2': _B_in['w2'], 'B_b2': _B_in['b2'], 'c': _w((lambda *s: _rng.normal(s) * 0.05)(8, 640)), 'w_mod': _w((lambda *s: _rng.normal(s) * 0.05)(640, 6 * 640) * 640 ** (-0.5))}

def reference(A_x, A_k_cache, A_v_cache, A_wq, A_wo, B_x, B_w1, B_b1, B_w2, B_b2, c, w_mod):

    def _A_ref(x, k_cache, v_cache, wq, wo):
        B, Sq, D = x.shape
        Hq, Dh = (32, 192)
        Hkv, Sk = (k_cache.shape[1], k_cache.shape[2])
        W = min(4096, max(256, Sk // 4))
        rep = Hq // Hkv
        q = (lambda x, *d: x.transpose(*d))((x @ wq).reshape(B, Sq, Hq, Dh), 0, 2, 1, 3)
        k = jnp.repeat(k_cache[:, :, Sk - W:, :], rep, axis=1)
        v = jnp.repeat(v_cache[:, :, Sk - W:, :], rep, axis=1)
        scores = jnp.einsum('bhqd,bhkd->bhqk', q, k) * Dh ** (-0.5)
        p = _softmax(scores, axis=-1)
        o = jnp.einsum('bhqk,bhkd->bhqd', p, v)
        return (lambda x, *d: x.transpose(*d))(o, 0, 2, 1, 3).reshape(B, Sq, Hq * Dh) @ wo

    def _B_ref(x, w1, b1, w2, b2):
        y = _layernorm(x, axis=-1)
        h = _gelu(jnp.einsum('bsd,df->bsf', y, w1) + b1)
        return jnp.einsum('bsf,fd->bsd', h, w2) + b2
    x = A_x
    mod = (_silu(c) @ w_mod).reshape(c.shape[0], 6, 1, -1)
    sa, ca, ga, sb, cb, gb = (mod[:, 0].copy(), mod[:, 1].copy(), mod[:, 2].copy(), mod[:, 3].copy(), mod[:, 4].copy(), mod[:, 5].copy())
    h = _layernorm(x, axis=-1) * (1 + ca) + sa
    x = x + ga * _A_ref(h, A_k_cache, A_v_cache, A_wq, A_wo)
    h = _layernorm(x, axis=-1) * (1 + cb) + sb
    x = x + gb * _B_ref(h, B_w1, B_b1, B_w2, B_b2)
    return x
```

```python
import functools

import jax
import jax.numpy as jnp
from jax import lax
import jax.experimental.pallas as pl
import jax.experimental.pallas.tpu as pltpu

_F32 = jnp.float32
_BF16 = jnp.bfloat16

_HQ = 32
_DH = 192
_HG = 8
_LANE = 128


def _layernorm(x, eps=1e-5):
    m = jnp.mean(x, axis=-1, keepdims=True)
    xc = x - m
    v = jnp.mean(xc * xc, axis=-1, keepdims=True)
    return xc / jnp.sqrt(v + eps)


def _gelu_tanh(x):
    return 0.5 * x * (1.0 + jnp.tanh(0.7978845608028654 * (x + 0.044715 * (x * x * x))))


def _dot(a, b):
    return jnp.dot(a, b, preferred_element_type=_F32)


def _dot_nt(a, b):
    return lax.dot_general(a, b, (((1,), (1,)), ((), ())), preferred_element_type=_F32)


def _kernel(x_hbm, k_hbm, v_hbm, wq_hbm, wo_hbm, w1_hbm, b1_hbm, w2_hbm, b2_hbm, c_hbm, wm_hbm,
            out_hbm,
            kbuf, vbuf, wm_buf, wq_buf, wo_buf, w1_buf, w2_buf,
            x_buf, c_buf, b1_buf, b2_buf, out_buf,
            h_scr, q_scr, o_scr, attn_scr,
            ksem, vsem, wsem,
            *, B, D, F, Sk, W, nslot, nch, nfc):
    G = _HQ // _HG
    R = _HG * _DH
    cw = W // nch
    nsteps = G * B
    fc = F // nfc

    def kv_copy(hbm, buf, sem, step, ch):
        g = step // B
        b = step % B
        slot = step % nslot
        return pltpu.make_async_copy(
            hbm.at[b * G + g, :, pl.ds(Sk - W + ch * cw, cw)],
            buf.at[slot, ch], sem.at[slot * nch + ch])

    def start_kv(step):
        for ch in range(nch):
            kv_copy(k_hbm, kbuf, ksem, step, ch).start()
        for ch in range(nch):
            kv_copy(v_hbm, vbuf, vsem, step, ch).start()

    S_X, S_C, S_B1, S_B2, S_OUT = 0, 1, 2, 3, 4
    S_WM = 5
    S_WQ = S_WM + 6
    S_WO = S_WQ + G
    S_W1 = S_WO + G
    S_W2 = S_W1 + nfc

    cp_x = pltpu.make_async_copy(x_hbm, x_buf, wsem.at[S_X])
    cp_c = pltpu.make_async_copy(c_hbm, c_buf, wsem.at[S_C])
    cp_b1 = pltpu.make_async_copy(b1_hbm, b1_buf, wsem.at[S_B1])
    cp_b2 = pltpu.make_async_copy(b2_hbm, b2_buf, wsem.at[S_B2])
    cp_out = pltpu.make_async_copy(out_buf, out_hbm, wsem.at[S_OUT])

    def cp_wm(j):
        return pltpu.make_async_copy(wm_hbm.at[:, pl.ds(j * D, D)], wm_buf.at[j], wsem.at[S_WM + j])

    def cp_wq(g):
        off = g * R if isinstance(g, int) else pl.multiple_of(g * R, _LANE)
        return pltpu.make_async_copy(wq_hbm.at[:, pl.ds(off, R)], wq_buf.at[g], wsem.at[S_WQ + g])

    def cp_wo(g):
        return pltpu.make_async_copy(wo_hbm.at[g], wo_buf.at[g], wsem.at[S_WO + g])

    def cp_w1(j):
        return pltpu.make_async_copy(w1_hbm.at[:, pl.ds(j * fc, fc)], w1_buf.at[j], wsem.at[S_W1 + j])

    def cp_w2(j):
        return pltpu.make_async_copy(w2_hbm.at[pl.ds(j * fc, fc), :], w2_buf.at[j], wsem.at[S_W2 + j])

    cp_wm(0).start()
    cp_wm(1).start()
    cp_c.start()
    cp_x.start()
    cp_wq(0).start()
    for s in range(nslot):
        start_kv(s)
    cp_b1.start()
    cp_b2.start()

    cp_c.wait()
    cp_x.wait()
    c = c_buf[...].astype(_F32)
    sc = (c * jax.nn.sigmoid(c)).astype(_BF16)
    x = x_buf[...].astype(_F32)
    ln_x = _layernorm(x)
    cp_wm(0).wait()
    sa = _dot(sc, wm_buf[0])
    cp_wm(1).wait()
    ca = _dot(sc, wm_buf[1])
    h_scr[...] = ln_x * (1.0 + ca) + sa
    attn_scr[...] = jnp.zeros_like(attn_scr)

    row = lax.broadcasted_iota(jnp.int32, (_HG, R), 0)
    col = lax.broadcasted_iota(jnp.int32, (_HG, R), 1)
    diag = (col >= row * _DH) & (col < (row + 1) * _DH)
    scale = float(_DH) ** -0.5

    def step_body(step, carry):
        g = step // B
        b = step % B
        slot = step % nslot

        @pl.when(b == 0)
        def _():
            cp_wq(g).wait()
            q = _dot(h_scr[...].astype(_BF16), wq_buf[g])
            q_scr[...] = q.astype(_BF16).astype(_F32)

        qrow = q_scr[pl.ds(b, 1), :]
        qbd = jnp.where(diag, jnp.broadcast_to(qrow, (_HG, R)), 0.0).astype(_BF16)
        s_parts = []
        for ch in range(nch):
            kv_copy(k_hbm, kbuf, ksem, step, ch).wait()
            s_parts.append(_dot(qbd, kbuf[slot, ch]))
        s = jnp.concatenate(s_parts, axis=-1) * scale
        m = jnp.max(s, axis=-1, keepdims=True)
        p = jnp.exp(s - m)
        l = jnp.sum(p, axis=-1, keepdims=True)
        pb = p.astype(_BF16)
        o = None
        for ch in range(nch):
            kv_copy(v_hbm, vbuf, vsem, step, ch).wait()
            part = _dot_nt(pb[:, ch * cw:(ch + 1) * cw], vbuf[slot, ch])
            o = part if o is None else o + part
        o = jnp.where(diag, o / l, 0.0)
        o_scr[pl.ds(b, 1), :] = jnp.sum(o, axis=0, keepdims=True)

        @pl.when(jnp.logical_and(b == 0, g + 1 < G))
        def _():
            cp_wq(g + 1).start()

        @pl.when(jnp.logical_and(b == 1, g + 1 < G))
        def _():
            cp_wo(g).start()

        @pl.when(step + nslot < nsteps)
        def _():
            start_kv(step + nslot)

        @pl.when(step + nslot == nsteps - 1)
        def _():
            cp_wo(G - 1).start()
            cp_wm(2).start()
            cp_wm(3).start()
            cp_wm(4).start()
            for j in range(nfc):
                cp_w1(j).start()
                cp_w2(j).start()
            cp_wm(5).start()

        @pl.when(b == B - 1)
        def _():
            cp_wo(g).wait()
            attn_scr[...] += _dot(o_scr[...].astype(_BF16), wo_buf[g])

        return carry

    lax.fori_loop(0, nsteps, step_body, 0)

    cp_wm(2).wait()
    ga = _dot(sc, wm_buf[2])
    x1 = x + ga * attn_scr[...]
    cp_wm(3).wait()
    sb = _dot(sc, wm_buf[3])
    cp_wm(4).wait()
    cb = _dot(sc, wm_buf[4])
    h2 = _layernorm(x1) * (1.0 + cb) + sb
    y = _layernorm(h2).astype(_BF16)
    cp_b1.wait()
    cp_b2.wait()
    b1 = b1_buf[...].astype(_F32)
    b2 = b2_buf[...].astype(_F32)
    mlp = jnp.concatenate([b2[i:i + 1, :] for i in range(D // _LANE)], axis=-1)
    tpc = fc // _LANE
    for j in range(nfc):
        cp_w1(j).wait()
        b1j = jnp.concatenate([b1[i:i + 1, :] for i in range(j * tpc, (j + 1) * tpc)], axis=-1)
        hj = _gelu_tanh(_dot(y, w1_buf[j]) + b1j).astype(_BF16)
        cp_w2(j).wait()
        mlp = mlp + _dot(hj, w2_buf[j])
    cp_wm(5).wait()
    gb = _dot(sc, wm_buf[5])
    out_buf[...] = (x1 + gb * mlp).astype(out_buf.dtype)
    cp_out.start()
    cp_out.wait()


def _run(A_x, A_k_cache, A_v_cache, A_wq, A_wo, B_w1, B_b1, B_w2, B_b2, c, w_mod,
         *, nslot=2, nch=4, nfc=3):
    B, Sq, D = A_x.shape
    _, Hkv, Sk, Dh = A_k_cache.shape
    F = B_w1.shape[1]
    assert Sq == 1 and Hkv == _HQ and Dh == _DH and B == 8
    W = min(4096, max(256, Sk // 4))
    G = _HQ // _HG
    R = _HG * _DH
    cw = W // nch
    fc = F // nfc

    x2 = A_x.reshape(B, D)
    kt = jnp.swapaxes(A_k_cache, 2, 3).reshape(B * G, R, Sk)
    vt = jnp.swapaxes(A_v_cache, 2, 3).reshape(B * G, R, Sk)
    wo = A_wo.reshape(G, R, D)
    b1 = B_b1.reshape(F // _LANE, _LANE)
    b2 = B_b2.reshape(D // _LANE, _LANE)

    kern = functools.partial(_kernel, B=B, D=D, F=F, Sk=Sk, W=W, nslot=nslot, nch=nch, nfc=nfc)
    any_spec = pl.BlockSpec(memory_space=pl.ANY)
    out = pl.pallas_call(
        kern,
        in_specs=[any_spec] * 11,
        out_specs=any_spec,
        out_shape=jax.ShapeDtypeStruct((B, D), A_x.dtype),
        scratch_shapes=[
            pltpu.VMEM((nslot, nch, R, cw), _BF16),
            pltpu.VMEM((nslot, nch, R, cw), _BF16),
            pltpu.VMEM((6, D, D), _BF16),
            pltpu.VMEM((G, D, R), _BF16),
            pltpu.VMEM((G, R, D), _BF16),
            pltpu.VMEM((nfc, D, fc), _BF16),
            pltpu.VMEM((nfc, fc, D), _BF16),
            pltpu.VMEM((B, D), _BF16),
            pltpu.VMEM((B, D), _BF16),
            pltpu.VMEM((F // _LANE, _LANE), _BF16),
            pltpu.VMEM((D // _LANE, _LANE), _BF16),
            pltpu.VMEM((B, D), A_x.dtype),
            pltpu.VMEM((B, D), _F32),
            pltpu.VMEM((B, R), _F32),
            pltpu.VMEM((B, R), _F32),
            pltpu.VMEM((B, D), _F32),
            pltpu.SemaphoreType.DMA((nslot * nch,)),
            pltpu.SemaphoreType.DMA((nslot * nch,)),
            pltpu.SemaphoreType.DMA((5 + 6 + 2 * G + 2 * nfc,)),
        ],
        compiler_params=pltpu.CompilerParams(vmem_limit_bytes=100 * 1024 * 1024),
    )(x2, kt, vt, A_wq, wo, B_w1, b1, B_w2, b2, c, w_mod)
    return out.reshape(B, Sq, D)


@jax.jit
def pallas_adaLN_cond__sliding_block_cached__mixer_channel_mlp__decode_kernel(
    A_x: jax.Array,
    A_k_cache: jax.Array,
    A_v_cache: jax.Array,
    A_wq: jax.Array,
    A_wo: jax.Array,
    B_x: jax.Array,
    B_w1: jax.Array,
    B_b1: jax.Array,
    B_w2: jax.Array,
    B_b2: jax.Array,
    c: jax.Array,
    w_mod: jax.Array,
):
    del B_x
    return _run(A_x, A_k_cache, A_v_cache, A_wq, A_wo, B_w1, B_b1, B_w2, B_b2, c, w_mod)
```

```python
import functools

import jax
import jax.numpy as jnp
from jax import lax
import jax.experimental.pallas as pl
import jax.experimental.pallas.tpu as pltpu

_F32 = jnp.float32
_BF16 = jnp.bfloat16

_HQ = 32
_DH = 192
_HG = 8
_LANE = 128


def _layernorm(x, eps=1e-5):
    m = jnp.mean(x, axis=-1, keepdims=True)
    xc = x - m
    v = jnp.mean(xc * xc, axis=-1, keepdims=True)
    return xc / jnp.sqrt(v + eps)


def _gelu_tanh(x):
    return 0.5 * x * (1.0 + jnp.tanh(0.7978845608028654 * (x + 0.044715 * (x * x * x))))


def _dot(a, b):
    return jnp.dot(a, b, preferred_element_type=_F32)


def _dot_nt(a, b):
    return lax.dot_general(a, b, (((1,), (1,)), ((), ())), preferred_element_type=_F32)


def _kernel(x_hbm, k_hbm, v_hbm, wq_hbm, wo_hbm, w1_hbm, b1_hbm, w2_hbm, b2_hbm, c_hbm, wm_hbm,
            out_hbm,
            kvbuf, wm_buf, wq_buf, wo_buf, w1_buf, w2_buf,
            x_buf, c_buf, b1_buf, b2_buf, out_buf,
            mod_scr, q_scr, o_scr, attn_scr,
            sem,
            *, B, D, F, Sk, W, cw, ur, hr, dl, dh, ns, fc, wsplit):
    G = _HQ // _HG
    R = _HG * _DH
    nc = W // cw
    nr = R // ur
    upb = nr * nc
    U = 2 * upb
    nsteps = G * B
    nfc = F // fc
    assert U % ns == 0 and dl <= ns and dh <= ns and dl <= U and dh <= U

    S_X, S_C, S_B1, S_B2, S_OUT = (2 * ns + i for i in range(5))

    def row_units(src, dst, rows, hrows, lo=0, hi=None):
        hi = src.shape[0] if hi is None else hi
        out = []
        for r in range(lo, hi, rows):
            a, b = pl.ds(r, rows - hrows), pl.ds(r + rows - hrows, hrows)
            out.append(((src.at[a, :], dst.at[a, :]), (src.at[b, :], dst.at[b, :])))
        return out

    wm_u = row_units(wm_hbm, wm_buf, *wsplit['wm'])
    wq_u = row_units(wq_hbm, wq_buf, *wsplit['wq'])
    wo_u = row_units(wo_hbm, wo_buf, *wsplit['wo'])
    pro = wm_u + wq_u + wo_u
    P = len(pro)
    epi = []
    epi_marks = []
    for j in range(nfc):
        w1s, w1d = w1_hbm.at[:, pl.ds(j * fc, fc)], w1_buf.at[j]
        epi += row_units(w1s, w1d, *wsplit['w1'])
        epi_marks.append(len(epi))
        epi += row_units(w2_hbm, w2_buf, *wsplit['w2'], lo=j * fc, hi=(j + 1) * fc)
        epi_marks.append(len(epi))
    E = len(epi)

    def kv_unit(step, u):
        isv, uu = divmod(u, upb)
        r, c = divmod(uu, nc)
        if isinstance(step, int):
            idx, slot = (step % B) * G + step // B, step % 2
        else:
            idx = lax.rem(step, B) * G + lax.div(step, B)
            slot = lax.rem(step, 2)
        src = (v_hbm if isv else k_hbm)
        lanes = pl.ds(Sk - W + c * cw, cw)
        a, b = pl.ds(r * ur, ur - hr), pl.ds((r + 1) * ur - hr, hr)
        return ((src.at[idx, a, lanes], kvbuf.at[slot, isv, c, a, :]),
                (src.at[idx, b, lanes], kvbuf.at[slot, isv, c, b, :]))

    def copy(unit, pos, cls):
        s, d = unit[cls]
        return pltpu.make_async_copy(s, d, sem.at[cls * ns + pos % ns])

    def start(unit, pos, cls):
        copy(unit, pos, cls).start(priority=1 - cls)

    def static_unit(pos):
        if pos < P:
            return pro[pos]
        if pos < P + nsteps * U:
            return kv_unit((pos - P) // U, (pos - P) % U)
        if pos < P + nsteps * U + E:
            return epi[pos - P - nsteps * U]
        return None

    def advance(cur, pos, nxt_h, nxt_l):
        copy(cur, pos, 0).wait()
        copy(cur, pos, 1).wait()
        if nxt_h is not None:
            start(nxt_h, pos + dh, 1)
        if nxt_l is not None:
            start(nxt_l, pos + dl, 0)

    def advance_static(pos):
        advance(static_unit(pos), pos, static_unit(pos + dh), static_unit(pos + dl))

    cp_x = pltpu.make_async_copy(x_hbm, x_buf, sem.at[S_X])
    cp_c = pltpu.make_async_copy(c_hbm, c_buf, sem.at[S_C])
    cp_b1 = pltpu.make_async_copy(b1_hbm, b1_buf, sem.at[S_B1])
    cp_b2 = pltpu.make_async_copy(b2_hbm, b2_buf, sem.at[S_B2])
    cp_out = pltpu.make_async_copy(out_buf, out_hbm, sem.at[S_OUT])

    for p in range(max(dl, dh)):
        if p < dl:
            start(static_unit(p), p, 0)
        if p < dh:
            start(static_unit(p), p, 1)
    cp_c.start()
    cp_x.start()
    cp_b1.start()
    cp_b2.start()

    pieces = {}

    def at(pos, fn):
        pieces.setdefault(pos, []).append(fn)

    def sc_val():
        c = c_buf[...].astype(_F32)
        return (c * jax.nn.sigmoid(c)).astype(_BF16)

    def wait_small():
        cp_c.wait()
        cp_x.wait()
        cp_b1.wait()
        cp_b2.wait()
        attn_scr[...] = jnp.zeros_like(attn_scr)
    at(len(wm_u) - 2, wait_small)

    def mod_piece(j):
        def f():
            mod_scr[j] = _dot(sc_val(), wm_buf[:, j * D:(j + 1) * D])
        return f
    for j in range(6):
        at(len(wm_u) - 1 + 2 * j, mod_piece(j))

    def h_piece():
        x = x_buf[...].astype(_F32)
        mod_scr[0] = _layernorm(x) * (1.0 + mod_scr[1]) + mod_scr[0]
    at(len(wm_u) + 12, h_piece)

    qw = 512
    def q_piece(j):
        def f():
            q = _dot(mod_scr[0].astype(_BF16), wq_buf[:, j * qw:(j + 1) * qw])
            g, o = divmod(j * qw, R)
            q_scr[g, :, o:o + qw] = q.astype(_BF16).astype(_F32)
        return f
    for j in range(_HQ * _DH // qw):
        at(len(wm_u) + len(wq_u) - 1 + j, q_piece(j))

    for p in range(P):
        advance_static(p)
        for f in pieces.get(p, []):
            f()

    row = lax.broadcasted_iota(jnp.int32, (_HG, R), 0)
    col = lax.broadcasted_iota(jnp.int32, (_HG, R), 1)
    diag = (col >= row * _DH) & (col < (row + 1) * _DH)
    scale = float(_DH) ** -0.5

    def attention_step(step, lookahead):
        if isinstance(step, int):
            g, b, slot = step // B, step % B, step % 2
        else:
            g, b, slot = lax.div(step, B), lax.rem(step, B), lax.rem(step, 2)
        qrow = q_scr[g, pl.ds(b, 1), :]
        qbd = jnp.where(diag, jnp.broadcast_to(qrow, (_HG, R)), 0.0).astype(_BF16)
        s_parts = [None] * nc
        o_parts = [None] * nr
        for u in range(U):
            isv, uu = divmod(u, upb)
            r, c = divmod(uu, nc)
            advance(kv_unit(step, u), P + u, lookahead(u + dh), lookahead(u + dl))
            blk = kvbuf[slot, isv, c, r * ur:(r + 1) * ur, :]
            if not isv:
                part = _dot(qbd[:, r * ur:(r + 1) * ur], blk)
                s_parts[c] = part if r == 0 else s_parts[c] + part
                if u == upb - 1:
                    s = jnp.concatenate(s_parts, axis=-1) * scale
                    m = jnp.max(s, axis=-1, keepdims=True)
                    p = jnp.exp(s - m)
                    l = jnp.sum(p, axis=-1, keepdims=True)
                    pb = p.astype(_BF16)
            else:
                part = _dot_nt(pb[:, c * cw:(c + 1) * cw], blk)
                o_parts[r] = part if c == 0 else o_parts[r] + part
        o = jnp.where(diag, jnp.concatenate(o_parts, axis=-1) / l, 0.0)
        o_scr[pl.ds(b, 1), :] = jnp.sum(o, axis=0, keepdims=True)

    def project(g):
        off = g * R if isinstance(g, int) else pl.multiple_of(g * R, R)
        attn_scr[...] += _dot(o_scr[...].astype(_BF16), wo_buf[pl.ds(off, R), :])

    def step_body(step, carry):
        attention_step(step, lambda u: kv_unit(step, u) if u < U else kv_unit(step + 1, u - U))

        @pl.when(lax.rem(step, B) == B - 1)
        def _():
            project(lax.div(step, B))
        return carry

    lax.fori_loop(0, nsteps - 1, step_body, 0)
    base = P + (nsteps - 1) * U
    attention_step(nsteps - 1, lambda u: static_unit(base + u))
    project(G - 1)

    base = P + nsteps * U
    x = x_buf[...].astype(_F32)
    x1 = x + mod_scr[2] * attn_scr[...]
    h2 = _layernorm(x1) * (1.0 + mod_scr[4]) + mod_scr[3]
    y = _layernorm(h2).astype(_BF16)
    b1 = b1_buf[...].astype(_F32)
    b2 = b2_buf[...].astype(_F32)
    mlp = jnp.concatenate([b2[i:i + 1, :] for i in range(D // _LANE)], axis=-1)
    tpc = fc // _LANE
    e = 0
    for j in range(nfc):
        while e < epi_marks[2 * j]:
            advance_static(base + e)
            e += 1
        b1j = jnp.concatenate([b1[i:i + 1, :] for i in range(j * tpc, (j + 1) * tpc)], axis=-1)
        hj = _gelu_tanh(_dot(y, w1_buf[j]) + b1j).astype(_BF16)
        while e < epi_marks[2 * j + 1]:
            advance_static(base + e)
            e += 1
        mlp = mlp + _dot(hj, w2_buf[j * fc:(j + 1) * fc, :])
    out_buf[...] = (x1 + mod_scr[5] * mlp).astype(out_buf.dtype)
    cp_out.start()
    cp_out.wait()


_WSPLIT = dict(wm=(32, 8), wq=(16, 8), wo=(128, 32), w1=(320, 80), w2=(128, 32))


def _run(A_x, A_k_cache, A_v_cache, A_wq, A_wo, B_w1, B_b1, B_w2, B_b2, c, w_mod,
         *, cw=256, ur=384, hr=96, dl=8, dh=8, ns=8, fc=256, wsplit=None):
    B, Sq, D = A_x.shape
    _, Hkv, Sk, Dh = A_k_cache.shape
    F = B_w1.shape[1]
    assert Sq == 1 and Hkv == _HQ and Dh == _DH and B == 8
    W = min(4096, max(256, Sk // 4))
    G = _HQ // _HG
    R = _HG * _DH
    ws = dict(_WSPLIT)
    ws.update(wsplit or {})

    x2 = A_x.reshape(B, D)
    kt = jnp.swapaxes(A_k_cache, 2, 3).reshape(B * G, R, Sk)
    vt = jnp.swapaxes(A_v_cache, 2, 3).reshape(B * G, R, Sk)
    b1 = B_b1.reshape(F // _LANE, _LANE)
    b2 = B_b2.reshape(D // _LANE, _LANE)

    kern = functools.partial(_kernel, B=B, D=D, F=F, Sk=Sk, W=W, cw=cw, ur=ur, hr=hr, dl=dl, dh=dh,
                             ns=ns, fc=fc, wsplit=ws)
    any_spec = pl.BlockSpec(memory_space=pl.ANY)
    out = pl.pallas_call(
        kern,
        in_specs=[any_spec] * 11,
        out_specs=any_spec,
        out_shape=jax.ShapeDtypeStruct((B, D), A_x.dtype),
        scratch_shapes=[
            pltpu.VMEM((2, 2, W // cw, R, cw), _BF16),
            pltpu.VMEM((D, 6 * D), _BF16),
            pltpu.VMEM((D, _HQ * _DH), _BF16),
            pltpu.VMEM((_HQ * _DH, D), _BF16),
            pltpu.VMEM((F // fc, D, fc), _BF16),
            pltpu.VMEM((F, D), _BF16),
            pltpu.VMEM((B, D), _BF16),
            pltpu.VMEM((B, D), _BF16),
            pltpu.VMEM((F // _LANE, _LANE), _BF16),
            pltpu.VMEM((D // _LANE, _LANE), _BF16),
            pltpu.VMEM((B, D), A_x.dtype),
            pltpu.VMEM((6, B, D), _F32),
            pltpu.VMEM((G, B, R), _F32),
            pltpu.VMEM((B, R), _F32),
            pltpu.VMEM((B, D), _F32),
            pltpu.SemaphoreType.DMA((2 * ns + 5,)),
        ],
        compiler_params=pltpu.CompilerParams(vmem_limit_bytes=100 * 1024 * 1024),
    )(x2, kt, vt, A_wq, A_wo, B_w1, b1, B_w2, b2, c, w_mod)
    return out.reshape(B, Sq, D)


@jax.jit
def pallas_adaLN_cond__sliding_block_cached__mixer_channel_mlp__decode_kernel(
    A_x: jax.Array,
    A_k_cache: jax.Array,
    A_v_cache: jax.Array,
    A_wq: jax.Array,
    A_wo: jax.Array,
    B_x: jax.Array,
    B_w1: jax.Array,
    B_b1: jax.Array,
    B_w2: jax.Array,
    B_b2: jax.Array,
    c: jax.Array,
    w_mod: jax.Array,
):
    del B_x
    return _run(A_x, A_k_cache, A_v_cache, A_wq, A_wo, B_w1, B_b1, B_w2, B_b2, c, w_mod)
```

```python
import functools

import jax
import jax.numpy as jnp
from jax import lax
import jax.experimental.pallas as pl
import jax.experimental.pallas.tpu as pltpu

_F32 = jnp.float32
_BF16 = jnp.bfloat16

_HQ = 32
_DH = 192
_HG = 8
_LANE = 128
_SUB = 8


def _layernorm(x, eps=1e-5):
    m = jnp.mean(x, axis=-1, keepdims=True)
    xc = x - m
    v = jnp.mean(xc * xc, axis=-1, keepdims=True)
    return xc / jnp.sqrt(v + eps)


def _gelu_tanh(x):
    return 0.5 * x * (1.0 + jnp.tanh(0.7978845608028654 * (x + 0.044715 * (x * x * x))))


def _dot(a, b):
    return jnp.dot(a, b, preferred_element_type=_F32)


def _dot_nt(a, b):
    return lax.dot_general(a, b, (((1,), (1,)), ((), ())), preferred_element_type=_F32)


def _spread(n_items, n_slots, first=0):
    out = {}
    span = n_slots - first
    for i in range(n_items):
        out.setdefault(first + (i * span) // n_items, []).append(i)
    return out


def _kernel(x_hbm, k_hbm, v_hbm, wq_hbm, wo_hbm, w1_hbm, b1_hbm, w2_hbm, b2_hbm, c_hbm, wm_hbm,
            out_hbm,
            kvbuf, wm_buf, wq_buf, wo_buf, w1_buf, w2_buf,
            x_buf, c_buf, b1_buf, b2_buf, out_buf,
            mod_scr, q_scr, o_scr, attn_scr,
            sem,
            *, B, D, F, Sk, W, cw, m, n, nh, pg, dl, dh, ns, fc, wsplit):
    G = _HQ // _HG
    R = _HG * _DH
    nc = W // cw
    GR = m * _SUB
    NG = R // GR
    rows_u = [(ph, g0) for ph in range(m) for g0 in range(0, NG, n)]
    blk_units = [(r, c) for r in rows_u for c in range(nc)]
    upb = len(blk_units)
    U = 2 * upb
    nsteps = G * B
    nfc = F // fc
    npc = NG // pg
    pr = pg * GR
    assert U % ns == 0 and dl <= ns and dh <= ns and dl <= upb and dh <= upb

    S_X, S_C, S_B1, S_B2, S_OUT = (2 * ns + i for i in range(5))

    def row_units(src, dst, rows, hrows, lo=0, hi=None):
        hi = src.shape[0] if hi is None else hi
        out = []
        for r in range(lo, hi, rows):
            a, b = pl.ds(r, rows - hrows), pl.ds(r + rows - hrows, hrows)
            out.append(((src.at[a, :], dst.at[a, :]), (src.at[b, :], dst.at[b, :])))
        return out

    wm_u = row_units(wm_hbm, wm_buf, *wsplit['wm'])
    wq_u = row_units(wq_hbm, wq_buf, *wsplit['wq'])
    wo_u = row_units(wo_hbm, wo_buf, *wsplit['wo'])
    pro = wm_u + wq_u + wo_u
    P = len(pro)
    epi = []
    epi_marks = []
    for j in range(nfc):
        w1s, w1d = w1_hbm.at[:, pl.ds(j * fc, fc)], w1_buf.at[j]
        epi += row_units(w1s, w1d, *wsplit['w1'])
        epi_marks.append(len(epi))
        epi += row_units(w2_hbm, w2_buf, *wsplit['w2'], lo=j * fc, hi=(j + 1) * fc)
        epi_marks.append(len(epi))
    E = len(epi)

    def split_step(step):
        if isinstance(step, int):
            return step // B, step % B, step % 2
        return lax.div(step, B), lax.rem(step, B), lax.rem(step, 2)

    def kv_unit(step, u):
        isv, uu = divmod(u, upb)
        (ph, g0), c = blk_units[uu]
        g, b, slot = split_step(step)
        idx = b * G + g
        src = (v_hbm if isv else k_hbm)
        lanes = pl.ds(Sk - W + c * cw, cw)
        rs = pl.ds(ph * _SUB, _SUB)
        lo, hi = pl.ds(g0, n - nh), pl.ds(g0 + n - nh, nh)
        return ((src.at[idx, lo, rs, lanes], kvbuf.at[slot, isv, c, lo, rs, :]),
                (src.at[idx, hi, rs, lanes], kvbuf.at[slot, isv, c, hi, rs, :]))

    def copy(unit, pos, cls):
        s, d = unit[cls]
        return pltpu.make_async_copy(s, d, sem.at[cls * ns + pos % ns])

    def start(unit, pos, cls):
        copy(unit, pos, cls).start(priority=1 - cls)

    def static_unit(pos):
        if pos < P:
            return pro[pos]
        if pos < P + nsteps * U:
            return kv_unit((pos - P) // U, (pos - P) % U)
        if pos < P + nsteps * U + E:
            return epi[pos - P - nsteps * U]
        return None

    def advance(cur, pos, nxt_h, nxt_l):
        copy(cur, pos, 0).wait()
        copy(cur, pos, 1).wait()
        if nxt_h is not None:
            start(nxt_h, pos + dh, 1)
        if nxt_l is not None:
            start(nxt_l, pos + dl, 0)

    def advance_static(pos):
        advance(static_unit(pos), pos, static_unit(pos + dh), static_unit(pos + dl))

    cp_x = pltpu.make_async_copy(x_hbm, x_buf, sem.at[S_X])
    cp_c = pltpu.make_async_copy(c_hbm, c_buf, sem.at[S_C])
    cp_b1 = pltpu.make_async_copy(b1_hbm, b1_buf, sem.at[S_B1])
    cp_b2 = pltpu.make_async_copy(b2_hbm, b2_buf, sem.at[S_B2])
    cp_out = pltpu.make_async_copy(out_buf, out_hbm, sem.at[S_OUT])

    for p in range(max(dl, dh)):
        if p < dl:
            start(static_unit(p), p, 0)
        if p < dh:
            start(static_unit(p), p, 1)
    cp_c.start()
    cp_x.start()
    cp_b1.start()
    cp_b2.start()

    pieces = {}

    def at(pos, fn):
        pieces.setdefault(pos, []).append(fn)

    def sc_val():
        c = c_buf[...].astype(_F32)
        return (c * jax.nn.sigmoid(c)).astype(_BF16)

    def wait_small():
        cp_c.wait()
        cp_x.wait()
        cp_b1.wait()
        cp_b2.wait()
        attn_scr[...] = jnp.zeros_like(attn_scr)
    at(len(wm_u) - 2, wait_small)

    def mod_piece(j):
        def f():
            mod_scr[j] = _dot(sc_val(), wm_buf[:, j * D:(j + 1) * D])
        return f
    for j in range(6):
        at(len(wm_u) - 1 + 2 * j, mod_piece(j))

    def h_piece():
        x = x_buf[...].astype(_F32)
        mod_scr[0] = _layernorm(x) * (1.0 + mod_scr[1]) + mod_scr[0]
    at(len(wm_u) + 12, h_piece)

    qw = 512

    def q_piece(j):
        def f():
            q = _dot(mod_scr[0].astype(_BF16), wq_buf[:, j * qw:(j + 1) * qw])
            g, o = divmod(j * qw, R)
            q_scr[g, :, o:o + qw] = q.astype(_BF16).astype(_F32)
        return f
    for j in range(_HQ * _DH // qw):
        at(len(wm_u) + len(wq_u) - 1 + 2 * j, q_piece(j))

    for p in range(P + upb):
        advance_static(p)
        for f in pieces.get(p, []):
            f()

    row = lax.broadcasted_iota(jnp.int32, (_HG, R), 0)
    col = lax.broadcasted_iota(jnp.int32, (_HG, R), 1)
    diag = (col >= row * _DH) & (col < (row + 1) * _DH)
    scale = float(_DH) ** -0.5

    def piece_rows(slot, isv, c, r):
        return kvbuf[slot, isv, c, r * pg:(r + 1) * pg].reshape(pr, cw)

    def scores_phase(step, adv):
        g, b, slot = split_step(step)
        sched = _spread(npc * nc, upb - 1)
        qrow = q_scr[g, pl.ds(b, 1), :]
        qbd = jnp.where(diag, jnp.broadcast_to(qrow, (_HG, R)), 0.0).astype(_BF16)
        parts = [None] * nc
        for u in range(upb):
            adv(u)
            for i in sched.get(u, []):
                r, c = divmod(i, nc)
                t = _dot(qbd[:, r * pr:(r + 1) * pr], piece_rows(slot, 0, c, r))
                parts[c] = t if r == 0 else parts[c] + t
        s = jnp.concatenate(parts, axis=-1) * scale
        mx = jnp.max(s, axis=-1, keepdims=True)
        p = jnp.exp(s - mx)
        l = jnp.sum(p, axis=-1, keepdims=True)
        return (p / l).astype(_BF16)

    def values_phase(step, pb, adv, nslots):
        g, b, slot = split_step(step)
        sched = _spread(npc * nc, nslots)
        parts = [None] * npc
        for u in range(nslots):
            adv(u)
            for i in sched.get(u, []):
                r, c = divmod(i, nc)
                t = _dot_nt(pb[:, c * cw:(c + 1) * cw], piece_rows(slot, 1, c, r))
                parts[r] = t if c == 0 else parts[r] + t
        o = jnp.where(diag, jnp.concatenate(parts, axis=-1), 0.0)
        o_scr[pl.ds(b, 1), :] = jnp.sum(o, axis=0, keepdims=True)

    def project(g):
        off = g * R if isinstance(g, int) else pl.multiple_of(g * R, R)
        attn_scr[...] += _dot(o_scr[...].astype(_BF16), wo_buf[pl.ds(off, R), :])

    def step_body(step, carry):
        def unit(u):
            return kv_unit(step, u) if u < U else kv_unit(step + 1, u - U)

        def adv(u):
            advance(unit(u), P + u, unit(u + dh), unit(u + dl))
        pb = scores_phase(step, lambda u: adv(upb + u))
        values_phase(step, pb, lambda u: adv(U + u), upb)

        @pl.when(lax.rem(step, B) == B - 1)
        def _():
            project(lax.div(step, B))
        return carry

    lax.fori_loop(0, nsteps - 1, step_body, 0)
    last = nsteps - 1
    pb = scores_phase(last, lambda u: advance_static(P + last * U + upb + u))
    base = P + nsteps * U
    e0 = min(E, wsplit['pv_slots'])
    values_phase(last, pb, lambda u: advance_static(base + u), e0)
    e = e0
    project(G - 1)

    x = x_buf[...].astype(_F32)
    x1 = x + mod_scr[2] * attn_scr[...]
    h2 = _layernorm(x1) * (1.0 + mod_scr[4]) + mod_scr[3]
    y = _layernorm(h2).astype(_BF16)
    b1 = b1_buf[...].astype(_F32)
    b2 = b2_buf[...].astype(_F32)
    mlp = jnp.concatenate([b2[i:i + 1, :] for i in range(D // _LANE)], axis=-1)
    tpc = fc // _LANE
    for j in range(nfc):
        while e < epi_marks[2 * j]:
            advance_static(base + e)
            e += 1
        b1j = jnp.concatenate([b1[i:i + 1, :] for i in range(j * tpc, (j + 1) * tpc)], axis=-1)
        hj = _gelu_tanh(_dot(y, w1_buf[j]) + b1j).astype(_BF16)
        while e < epi_marks[2 * j + 1]:
            advance_static(base + e)
            e += 1
        mlp = mlp + _dot(hj, w2_buf[j * fc:(j + 1) * fc, :])
    out_buf[...] = (x1 + mod_scr[5] * mlp).astype(out_buf.dtype)
    cp_out.start()
    cp_out.wait()


_WSPLIT = dict(wm=(32, 8), wq=(16, 8), wo=(128, 32), w1=(320, 80), w2=(128, 32), pv_slots=6)


def _run(A_x, A_k_cache, A_v_cache, A_wq, A_wo, B_w1, B_b1, B_w2, B_b2, c, w_mod,
         *, cw=256, m=6, n=16, nh=2, pg=8, dl=16, dh=16, ns=16, fc=256, wsplit=None,
         nobc=True, nosc=True):
    B, Sq, D = A_x.shape
    _, Hkv, Sk, Dh = A_k_cache.shape
    F = B_w1.shape[1]
    assert Sq == 1 and Hkv == _HQ and Dh == _DH and B == 8
    W = min(4096, max(256, Sk // 4))
    G = _HQ // _HG
    R = _HG * _DH
    GR = m * _SUB
    ws = dict(_WSPLIT)
    ws.update(wsplit or {})

    x2 = A_x.reshape(B, D)
    kt = jnp.swapaxes(A_k_cache, 2, 3).reshape(B * G, R // GR, GR, Sk)
    vt = jnp.swapaxes(A_v_cache, 2, 3).reshape(B * G, R // GR, GR, Sk)
    b1 = B_b1.reshape(F // _LANE, _LANE)
    b2 = B_b2.reshape(D // _LANE, _LANE)

    kern = functools.partial(_kernel, B=B, D=D, F=F, Sk=Sk, W=W, cw=cw, m=m, n=n, nh=nh, pg=pg,
                             dl=dl, dh=dh, ns=ns, fc=fc, wsplit=ws)
    any_spec = pl.BlockSpec(memory_space=pl.ANY)
    out = pl.pallas_call(
        kern,
        in_specs=[any_spec] * 11,
        out_specs=any_spec,
        out_shape=jax.ShapeDtypeStruct((B, D), A_x.dtype),
        scratch_shapes=[
            pltpu.VMEM((2, 2, W // cw, R // GR, GR, cw), _BF16),
            pltpu.VMEM((D, 6 * D), _BF16),
            pltpu.VMEM((D, _HQ * _DH), _BF16),
            pltpu.VMEM((_HQ * _DH, D), _BF16),
            pltpu.VMEM((F // fc, D, fc), _BF16),
            pltpu.VMEM((F, D), _BF16),
            pltpu.VMEM((B, D), _BF16),
            pltpu.VMEM((B, D), _BF16),
            pltpu.VMEM((F // _LANE, _LANE), _BF16),
            pltpu.VMEM((D // _LANE, _LANE), _BF16),
            pltpu.VMEM((B, D), A_x.dtype),
            pltpu.VMEM((6, B, D), _F32),
            pltpu.VMEM((G, B, R), _F32),
            pltpu.VMEM((B, R), _F32),
            pltpu.VMEM((B, D), _F32),
            pltpu.SemaphoreType.DMA((2 * ns + 5,)),
        ],
        compiler_params=pltpu.CompilerParams(vmem_limit_bytes=100 * 1024 * 1024, disable_bounds_checks=nobc,
                                             disable_semaphore_checks=nosc),
    )(x2, kt, vt, A_wq, A_wo, B_w1, b1, B_w2, b2, c, w_mod)
    return out.reshape(B, Sq, D)


@jax.jit
def pallas_adaLN_cond__sliding_block_cached__mixer_channel_mlp__decode_kernel(
    A_x: jax.Array,
    A_k_cache: jax.Array,
    A_v_cache: jax.Array,
    A_wq: jax.Array,
    A_wo: jax.Array,
    B_x: jax.Array,
    B_w1: jax.Array,
    B_b1: jax.Array,
    B_w2: jax.Array,
    B_b2: jax.Array,
    c: jax.Array,
    w_mod: jax.Array,
):
    del B_x
    return _run(A_x, A_k_cache, A_v_cache, A_wq, A_wo, B_w1, B_b1, B_w2, B_b2, c, w_mod)
```

```python
import functools

import jax
import jax.numpy as jnp
from jax import lax
import jax.experimental.pallas as pl
import jax.experimental.pallas.tpu as pltpu

_F32 = jnp.float32
_BF16 = jnp.bfloat16

_HQ = 32
_DH = 192
_HG = 8
_LANE = 128
_SUB = 8


def _layernorm(x, eps=1e-5):
    m = jnp.mean(x, axis=-1, keepdims=True)
    xc = x - m
    v = jnp.mean(xc * xc, axis=-1, keepdims=True)
    return xc / jnp.sqrt(v + eps)


def _gelu_tanh(x):
    return 0.5 * x * (1.0 + jnp.tanh(0.7978845608028654 * (x + 0.044715 * (x * x * x))))


def _dot(a, b):
    return jnp.dot(a, b, preferred_element_type=_F32)


def _dot_nt(a, b):
    return lax.dot_general(a, b, (((1,), (1,)), ((), ())), preferred_element_type=_F32)


def _spread(n_items, n_slots, first=0):
    out = {}
    span = n_slots - first
    for i in range(n_items):
        out.setdefault(first + (i * span) // n_items, []).append(i)
    return out


def _kernel(x_hbm, k_hbm, v_hbm, wq_hbm, wo_hbm, w1_hbm, b1_hbm, w2_hbm, b2_hbm, c_hbm, wm_hbm,
            out_hbm,
            kvbuf, wm_buf, wq_buf, wo_buf, w1_buf, w2_buf,
            x_buf, c_buf, b1_buf, b2_buf, out_buf,
            mod_scr, q_scr, o_scr, attn_scr,
            sem,
            *, B, D, F, Sk, W, cw, m, n, nh, pg, ps, dl, dh, ns, fc, wsplit):
    G = _HQ // _HG
    R = _HG * _DH
    nc = W // cw
    GR = m * _SUB
    NG = R // GR
    rows_u = [(ph, g0) for ph in range(m) for g0 in range(0, NG, n)]
    blk_units = [(r, c) for r in rows_u for c in range(nc)]
    upb = len(blk_units)
    U = 2 * upb
    nsteps = G * B
    nfc = F // fc
    npc = NG // pg
    pr = pg * GR
    assert U % ns == 0 and dl <= ns and dh <= ns and dl <= upb and dh <= upb

    S_X, S_C, S_B1, S_B2, S_OUT = (2 * ns + i for i in range(5))

    def strided_units(src, dst, g_lo, g_hi, n_, nh_, cw_, rr=_SUB):
        out = []
        for r in range(0, src.shape[1], rr):
            for g0 in range(g_lo, g_hi, n_):
                for c0 in range(0, src.shape[2], cw_):
                    rs, cs = pl.ds(r, rr), pl.ds(c0, cw_)
                    lo, hi = pl.ds(g0, n_ - nh_), pl.ds(g0 + n_ - nh_, nh_)
                    out.append(((src.at[lo, rs, cs], dst.at[lo, rs, cs]),
                                (src.at[hi, rs, cs], dst.at[hi, rs, cs])))
        return out

    def seq_units(src, dst, g, rows, hrows):
        out = []
        for r in range(0, src.shape[1], rows):
            lo, hi = pl.ds(r, rows - hrows), pl.ds(r + rows - hrows, hrows)
            out.append(((src.at[g, lo, :], dst.at[g, lo, :]), (src.at[g, hi, :], dst.at[g, hi, :])))
        return out

    gpo = wo_hbm.shape[0] // G
    wm_u = strided_units(wm_hbm, wm_buf, 0, wm_hbm.shape[0], *wsplit['wm'])
    wq_u = strided_units(wq_hbm, wq_buf, 0, wq_hbm.shape[0], *wsplit['wq'])
    wo_u = strided_units(wo_hbm, wo_buf, 0, (G - 1) * gpo, *wsplit['wo'])
    pro = wm_u + wq_u + wo_u
    P = len(pro)
    wo3_u = strided_units(wo_hbm, wo_buf, (G - 1) * gpo, G * gpo, *wsplit['wo3'])
    w1_u = strided_units(w1_hbm, w1_buf, 0, w1_hbm.shape[0], *wsplit['w1'])
    w2_u = seq_units(w2_hbm, w2_buf, 0, *wsplit['w2'])
    epi = wo3_u + w1_u + w2_u
    E = len(epi)

    def split_step(step):
        if isinstance(step, int):
            return step // B, step % B, step % 2
        return lax.div(step, B), lax.rem(step, B), lax.rem(step, 2)

    def kv_unit(step, u):
        isv, uu = divmod(u, upb)
        (ph, g0), c = blk_units[uu]
        g, b, slot = split_step(step)
        idx = b * G + g
        src = (v_hbm if isv else k_hbm)
        lanes = pl.ds(Sk - W + c * cw, cw)
        rs = pl.ds(ph * _SUB, _SUB)
        lo, hi = pl.ds(g0, n - nh), pl.ds(g0 + n - nh, nh)
        return ((src.at[idx, lo, rs, lanes], kvbuf.at[slot, isv, c, lo, rs, :]),
                (src.at[idx, hi, rs, lanes], kvbuf.at[slot, isv, c, hi, rs, :]))

    def copy(unit, pos, cls):
        s, d = unit[cls]
        return pltpu.make_async_copy(s, d, sem.at[cls * ns + pos % ns])

    def start(unit, pos, cls):
        copy(unit, pos, cls).start(priority=1 - cls)

    def static_unit(pos):
        if pos < P:
            return pro[pos]
        if pos < P + nsteps * U:
            return kv_unit((pos - P) // U, (pos - P) % U)
        if pos < P + nsteps * U + E:
            return epi[pos - P - nsteps * U]
        return None

    def advance(cur, pos, nxt_h, nxt_l):
        copy(cur, pos, 0).wait()
        copy(cur, pos, 1).wait()
        if nxt_h is not None:
            start(nxt_h, pos + dh, 1)
        if nxt_l is not None:
            start(nxt_l, pos + dl, 0)

    def advance_static(pos):
        advance(static_unit(pos), pos, static_unit(pos + dh), static_unit(pos + dl))

    cp_x = pltpu.make_async_copy(x_hbm, x_buf, sem.at[S_X])
    cp_c = pltpu.make_async_copy(c_hbm, c_buf, sem.at[S_C])
    cp_b1 = pltpu.make_async_copy(b1_hbm, b1_buf, sem.at[S_B1])
    cp_b2 = pltpu.make_async_copy(b2_hbm, b2_buf, sem.at[S_B2])
    cp_out = pltpu.make_async_copy(out_buf, out_hbm, sem.at[S_OUT])

    for p in range(max(dl, dh)):
        if p < dl:
            start(static_unit(p), p, 0)
        if p < dh:
            start(static_unit(p), p, 1)
    cp_c.start()
    cp_x.start()
    cp_b1.start()
    cp_b2.start()

    pieces = {}

    def at(pos, fn):
        pieces.setdefault(pos, []).append(fn)

    def sc_val():
        c = c_buf[...].astype(_F32)
        return (c * jax.nn.sigmoid(c)).astype(_BF16)

    def wait_small():
        cp_c.wait()
        cp_x.wait()
        cp_b1.wait()
        cp_b2.wait()
        attn_scr[...] = jnp.zeros_like(attn_scr)
    at(len(wm_u) - 2, wait_small)

    def mod_piece(j):
        def f():
            mod_scr[j] = _dot(sc_val(), wm_buf[:, :, j * D:(j + 1) * D].reshape(D, D))
        return f
    for j in range(6):
        at(len(wm_u) - 1 + 4 * j, mod_piece(j))

    def h_piece():
        x = x_buf[...].astype(_F32)
        mod_scr[0] = _layernorm(x) * (1.0 + mod_scr[1]) + mod_scr[0]
    at(len(wm_u) + 24, h_piece)

    qw = 512

    def q_piece(j):
        def f():
            q = _dot(mod_scr[0].astype(_BF16), wq_buf[:, :, j * qw:(j + 1) * qw].reshape(D, qw))
            g, o = divmod(j * qw, R)
            q_scr[g, :, o:o + qw] = q.astype(_BF16).astype(_F32)
        return f
    for j in range(_HQ * _DH // qw):
        at(len(wm_u) + len(wq_u) - 1 + 3 * j, q_piece(j))

    for p in range(P + upb):
        advance_static(p)
        for f in pieces.get(p, []):
            f()

    row = lax.broadcasted_iota(jnp.int32, (_HG, R), 0)
    col = lax.broadcasted_iota(jnp.int32, (_HG, R), 1)
    diag = (col >= row * _DH) & (col < (row + 1) * _DH)
    scale = float(_DH) ** -0.5

    pw = cw // ps
    npl = nc * ps

    def piece_rows(slot, isv, c, r):
        cc, j = divmod(c, ps)
        return kvbuf[slot, isv, cc, r * pg:(r + 1) * pg, :, j * pw:(j + 1) * pw].reshape(pr, pw)

    def scores_phase(step, adv):
        g, b, slot = split_step(step)
        sched = _spread(npc * npl, upb - 1)
        qrow = q_scr[g, pl.ds(b, 1), :]
        qbd = jnp.where(diag, jnp.broadcast_to(qrow, (_HG, R)), 0.0).astype(_BF16)
        parts = [None] * npl
        for u in range(upb):
            adv(u)
            for i in sched.get(u, []):
                r, c = divmod(i, npl)
                t = _dot(qbd[:, r * pr:(r + 1) * pr], piece_rows(slot, 0, c, r))
                parts[c] = t if r == 0 else parts[c] + t
        s = jnp.concatenate(parts, axis=-1) * scale
        mx = jnp.max(s, axis=-1, keepdims=True)
        p = jnp.exp(s - mx)
        l = jnp.sum(p, axis=-1, keepdims=True)
        return (p / l).astype(_BF16)

    def values_phase(step, pb, adv, nslots):
        g, b, slot = split_step(step)
        sched = _spread(npc * npl, nslots)
        parts = [None] * npc
        for u in range(nslots):
            adv(u)
            for i in sched.get(u, []):
                r, c = divmod(i, npl)
                t = _dot_nt(pb[:, c * pw:(c + 1) * pw], piece_rows(slot, 1, c, r))
                parts[r] = t if c == 0 else parts[r] + t
        o = jnp.where(diag, jnp.concatenate(parts, axis=-1), 0.0)
        o_scr[pl.ds(b, 1), :] = jnp.sum(o, axis=0, keepdims=True)

    def project(g):
        attn_scr[...] += _dot(o_scr[...].astype(_BF16), wo_buf[pl.ds(g * gpo, gpo)].reshape(R, D))

    def step_body(step, carry):
        def unit(u):
            return kv_unit(step, u) if u < U else kv_unit(step + 1, u - U)

        def adv(u):
            advance(unit(u), P + u, unit(u + dh), unit(u + dl))
        pb = scores_phase(step, lambda u: adv(upb + u))
        values_phase(step, pb, lambda u: adv(U + u), upb)

        @pl.when(lax.rem(step, B) == B - 1)
        def _():
            project(lax.div(step, B))
        return carry

    lax.fori_loop(0, nsteps - 1, step_body, 0)
    last = nsteps - 1
    pb = scores_phase(last, lambda u: advance_static(P + last * U + upb + u))
    base = P + nsteps * U
    values_phase(last, pb, lambda u: advance_static(base + u), len(wo3_u))
    cur = [len(wo3_u)]

    def run_to(mark):
        while cur[0] < mark:
            advance_static(base + cur[0])
            cur[0] += 1

    project(G - 1)
    run_to(cur[0] + wsplit['gap'])

    x = x_buf[...].astype(_F32)
    x1 = x + mod_scr[2] * attn_scr[...]
    h2 = _layernorm(x1) * (1.0 + mod_scr[4]) + mod_scr[3]
    y = _layernorm(h2).astype(_BF16)
    b1 = b1_buf[...].astype(_F32)
    b2 = b2_buf[...].astype(_F32)
    mlp = jnp.concatenate([b2[i:i + 1, :] for i in range(D // _LANE)], axis=-1)
    run_to(len(wo3_u) + len(w1_u))
    hs = []
    tpc = fc // _LANE
    for j in range(nfc):
        b1j = jnp.concatenate([b1[i:i + 1, :] for i in range(j * tpc, (j + 1) * tpc)], axis=-1)
        hs.append(_gelu_tanh(_dot(y, w1_buf[:, :, j * fc:(j + 1) * fc].reshape(D, fc)) + b1j).astype(_BF16))
        run_to(cur[0] + wsplit['gap2'])
    hh = jnp.concatenate(hs, axis=-1)
    done = 0
    for have in wsplit['w2marks']:
        run_to(E - len(w2_u) + have // wsplit['w2'][0])
        mlp = mlp + _dot(hh[:, done:have], w2_buf[0, done:have, :])
        done = have
    out_buf[...] = (x1 + mod_scr[5] * mlp).astype(out_buf.dtype)
    cp_out.start()
    cp_out.wait()


_WSPLIT = dict(wm=(8, 2, 640), wq=(8, 2, 768), wo=(6, 1, 640), wo3=(4, 1, 640, 16), w1=(4, 1, 1536),
               w2=(64, 16), w2marks=(768, 1152, 1408, 1536), gap=4, gap2=3,
               rm=80, rq=80, ro=384, r1=160, r2=1536)


def _run(A_x, A_k_cache, A_v_cache, A_wq, A_wo, B_w1, B_b1, B_w2, B_b2, c, w_mod,
         *, cw=256, m=6, n=16, nh=2, pg=8, ps=1, dl=24, dh=12, ns=24, fc=512, wsplit=None,
         nobc=True, nosc=True):
    B, Sq, D = A_x.shape
    _, Hkv, Sk, Dh = A_k_cache.shape
    F = B_w1.shape[1]
    assert Sq == 1 and Hkv == _HQ and Dh == _DH and B == 8
    W = min(4096, max(256, Sk // 4))
    G = _HQ // _HG
    R = _HG * _DH
    GR = m * _SUB
    ws = dict(_WSPLIT)
    ws.update(wsplit or {})

    x2 = A_x.reshape(B, D)
    kt = jnp.swapaxes(A_k_cache, 2, 3).reshape(B * G, R // GR, GR, Sk)
    vt = jnp.swapaxes(A_v_cache, 2, 3).reshape(B * G, R // GR, GR, Sk)
    wm = w_mod.reshape(-1, ws['rm'], w_mod.shape[1])
    wq = A_wq.reshape(-1, ws['rq'], A_wq.shape[1])
    wo = A_wo.reshape(-1, ws['ro'], D)
    w1 = B_w1.reshape(-1, ws['r1'], F)
    w2 = B_w2.reshape(-1, ws['r2'], D)
    b1 = B_b1.reshape(F // _LANE, _LANE)
    b2 = B_b2.reshape(D // _LANE, _LANE)

    kern = functools.partial(_kernel, B=B, D=D, F=F, Sk=Sk, W=W, cw=cw, m=m, n=n, nh=nh, pg=pg, ps=ps,
                             dl=dl, dh=dh, ns=ns, fc=fc, wsplit=ws)
    any_spec = pl.BlockSpec(memory_space=pl.ANY)
    out = pl.pallas_call(
        kern,
        in_specs=[any_spec] * 11,
        out_specs=any_spec,
        out_shape=jax.ShapeDtypeStruct((B, D), A_x.dtype),
        scratch_shapes=[
            pltpu.VMEM((2, 2, W // cw, R // GR, GR, cw), _BF16),
            pltpu.VMEM(wm.shape, _BF16),
            pltpu.VMEM(wq.shape, _BF16),
            pltpu.VMEM(wo.shape, _BF16),
            pltpu.VMEM(w1.shape, _BF16),
            pltpu.VMEM(w2.shape, _BF16),
            pltpu.VMEM((B, D), _BF16),
            pltpu.VMEM((B, D), _BF16),
            pltpu.VMEM((F // _LANE, _LANE), _BF16),
            pltpu.VMEM((D // _LANE, _LANE), _BF16),
            pltpu.VMEM((B, D), A_x.dtype),
            pltpu.VMEM((6, B, D), _F32),
            pltpu.VMEM((G, B, R), _F32),
            pltpu.VMEM((B, R), _F32),
            pltpu.VMEM((B, D), _F32),
            pltpu.SemaphoreType.DMA((2 * ns + 5,)),
        ],
        compiler_params=pltpu.CompilerParams(vmem_limit_bytes=100 * 1024 * 1024, disable_bounds_checks=nobc,
                                             disable_semaphore_checks=nosc),
    )(x2, kt, vt, wq, wo, w1, b1, w2, b2, c, wm)
    return out.reshape(B, Sq, D)


@jax.jit
def pallas_adaLN_cond__sliding_block_cached__mixer_channel_mlp__decode_kernel(
    A_x: jax.Array,
    A_k_cache: jax.Array,
    A_v_cache: jax.Array,
    A_wq: jax.Array,
    A_wo: jax.Array,
    B_x: jax.Array,
    B_w1: jax.Array,
    B_b1: jax.Array,
    B_w2: jax.Array,
    B_b2: jax.Array,
    c: jax.Array,
    w_mod: jax.Array,
):
    del B_x
    return _run(A_x, A_k_cache, A_v_cache, A_wq, A_wo, B_w1, B_b1, B_w2, B_b2, c, w_mod)
```

```python
import functools

import jax
import jax.numpy as jnp
from jax import lax
import jax.experimental.pallas as pl
import jax.experimental.pallas.tpu as pltpu

_F32 = jnp.float32
_BF16 = jnp.bfloat16

_HQ = 32
_DH = 192
_HG = 8
_LANE = 128
_SUB = 8


def _layernorm(x, eps=1e-5):
    m = jnp.mean(x, axis=-1, keepdims=True)
    xc = x - m
    v = jnp.mean(xc * xc, axis=-1, keepdims=True)
    return xc / jnp.sqrt(v + eps)


def _gelu_tanh(x):
    return 0.5 * x * (1.0 + jnp.tanh(0.7978845608028654 * (x + 0.044715 * (x * x * x))))


def _dot(a, b):
    return jnp.dot(a, b, preferred_element_type=_F32)


def _dot_nt(a, b):
    return lax.dot_general(a, b, (((1,), (1,)), ((), ())), preferred_element_type=_F32)


def _spread(n_items, n_slots, first=0):
    out = {}
    span = n_slots - first
    for i in range(n_items):
        out.setdefault(first + (i * span) // n_items, []).append(i)
    return out


def _kernel(x_hbm, k_hbm, v_hbm, wq_hbm, wo_hbm, w1_hbm, b1_hbm, w2_hbm, b2_hbm, c_hbm, wm_hbm,
            out_hbm,
            kvbuf, wm_buf, wq_buf, wo_buf, w1_buf, w2_buf,
            x_buf, c_buf, b1_buf, b2_buf, out_buf,
            mod_scr, q_scr, o_scr, attn_scr,
            sem,
            *, B, D, F, Sk, W, cw, m, n, nh, corder, pg, ps, dl, dh, ns, fc, wsplit):
    G = _HQ // _HG
    R = _HG * _DH
    nc = W // cw
    GR = m * _SUB
    NG = R // GR
    rows_u = [(ph, g0) for ph in range(m) for g0 in range(0, NG, n)]
    blk_units = [(r, c) for r in rows_u for c in corder]
    upb = len(blk_units)
    U = 2 * upb
    nsteps = G * B
    nfc = F // fc
    npc = NG // pg
    pr = pg * GR
    assert U % ns == 0 and dl <= ns and dh <= ns and dl <= upb and dh <= upb

    S_X, S_C, S_B1, S_B2, S_OUT = (2 * ns + i for i in range(5))

    def strided_units(src, dst, g_lo, g_hi, n_, nh_, cw_, rr=_SUB):
        out = []
        for r in range(0, src.shape[1], rr):
            for g0 in range(g_lo, g_hi, n_):
                for c0 in range(0, src.shape[2], cw_):
                    rs, cs = pl.ds(r, rr), pl.ds(c0, cw_)
                    lo, hi = pl.ds(g0, n_ - nh_), pl.ds(g0 + n_ - nh_, nh_)
                    out.append(((src.at[lo, rs, cs], dst.at[lo, rs, cs]),
                                (src.at[hi, rs, cs], dst.at[hi, rs, cs])))
        return out

    def seq_units(src, dst, g, rows, hrows):
        out = []
        for r in range(0, src.shape[1], rows):
            lo, hi = pl.ds(r, rows - hrows), pl.ds(r + rows - hrows, hrows)
            out.append(((src.at[g, lo, :], dst.at[g, lo, :]), (src.at[g, hi, :], dst.at[g, hi, :])))
        return out

    gpo = wo_hbm.shape[0] // G
    wm_u = strided_units(wm_hbm, wm_buf, 0, wm_hbm.shape[0], *wsplit['wm'])
    wq_u = strided_units(wq_hbm, wq_buf, 0, wq_hbm.shape[0], *wsplit['wq'])
    wo_u = strided_units(wo_hbm, wo_buf, 0, (G - 1) * gpo, *wsplit['wo'])
    pro = wm_u + wq_u + wo_u
    P = len(pro)
    wo3_u = strided_units(wo_hbm, wo_buf, (G - 1) * gpo, G * gpo, *wsplit['wo3'])
    w1_u = strided_units(w1_hbm, w1_buf, 0, w1_hbm.shape[0], *wsplit['w1'])
    w2_u = seq_units(w2_hbm, w2_buf, 0, *wsplit['w2'])
    epi = wo3_u + w1_u + w2_u
    E = len(epi)

    def split_step(step):
        if isinstance(step, int):
            return step // B, step % B, step % 2
        return lax.div(step, B), lax.rem(step, B), lax.rem(step, 2)

    def kv_unit(step, u):
        isv, uu = divmod(u, upb)
        (ph, g0), c = blk_units[uu]
        g, b, slot = split_step(step)
        idx = b * G + g
        src = (v_hbm if isv else k_hbm)
        lanes = pl.ds(Sk - W + c * cw, cw)
        rs = pl.ds(ph * _SUB, _SUB)
        lo, hi = pl.ds(g0, n - nh), pl.ds(g0 + n - nh, nh)
        return ((src.at[idx, lo, rs, lanes], kvbuf.at[slot, isv, c, lo, rs, :]),
                (src.at[idx, hi, rs, lanes], kvbuf.at[slot, isv, c, hi, rs, :]))

    def copy(unit, pos, cls):
        s, d = unit[cls]
        return pltpu.make_async_copy(s, d, sem.at[cls * ns + pos % ns])

    def start(unit, pos, cls):
        copy(unit, pos, cls).start(priority=1 - cls)

    def static_unit(pos):
        if pos < P:
            return pro[pos]
        if pos < P + nsteps * U:
            return kv_unit((pos - P) // U, (pos - P) % U)
        if pos < P + nsteps * U + E:
            return epi[pos - P - nsteps * U]
        return None

    def advance(cur, pos, nxt_h, nxt_l):
        copy(cur, pos, 0).wait()
        copy(cur, pos, 1).wait()
        if nxt_h is not None:
            start(nxt_h, pos + dh, 1)
        if nxt_l is not None:
            start(nxt_l, pos + dl, 0)

    def advance_static(pos):
        advance(static_unit(pos), pos, static_unit(pos + dh), static_unit(pos + dl))

    cp_x = pltpu.make_async_copy(x_hbm, x_buf, sem.at[S_X])
    cp_c = pltpu.make_async_copy(c_hbm, c_buf, sem.at[S_C])
    cp_b1 = pltpu.make_async_copy(b1_hbm, b1_buf, sem.at[S_B1])
    cp_b2 = pltpu.make_async_copy(b2_hbm, b2_buf, sem.at[S_B2])
    cp_out = pltpu.make_async_copy(out_buf, out_hbm, sem.at[S_OUT])

    for p in range(max(dl, dh)):
        if p < dl:
            start(static_unit(p), p, 0)
        if p < dh:
            start(static_unit(p), p, 1)
    cp_c.start()
    cp_x.start()
    cp_b1.start()
    cp_b2.start()

    pieces = {}

    def at(pos, fn):
        pieces.setdefault(pos, []).append(fn)

    def sc_val():
        c = c_buf[...].astype(_F32)
        return (c * jax.nn.sigmoid(c)).astype(_BF16)

    def wait_small():
        cp_c.wait()
        cp_x.wait()
        cp_b1.wait()
        cp_b2.wait()
        attn_scr[...] = jnp.zeros_like(attn_scr)
    at(len(wm_u) - 2, wait_small)

    def mod_piece(j):
        def f():
            mod_scr[j] = _dot(sc_val(), wm_buf[:, :, j * D:(j + 1) * D].reshape(D, D))
        return f
    for j in range(6):
        at(len(wm_u) - 1 + 4 * j, mod_piece(j))

    def h_piece():
        x = x_buf[...].astype(_F32)
        mod_scr[0] = _layernorm(x) * (1.0 + mod_scr[1]) + mod_scr[0]
    at(len(wm_u) + 24, h_piece)

    qw = 512

    def q_piece(j):
        def f():
            q = _dot(mod_scr[0].astype(_BF16), wq_buf[:, :, j * qw:(j + 1) * qw].reshape(D, qw))
            g, o = divmod(j * qw, R)
            q_scr[g, :, o:o + qw] = q.astype(_BF16).astype(_F32)
        return f
    for j in range(_HQ * _DH // qw):
        at(len(wm_u) + len(wq_u) - 1 + 3 * j, q_piece(j))

    for p in range(P + upb):
        advance_static(p)
        for f in pieces.get(p, []):
            f()

    row = lax.broadcasted_iota(jnp.int32, (_HG, R), 0)
    col = lax.broadcasted_iota(jnp.int32, (_HG, R), 1)
    diag = (col >= row * _DH) & (col < (row + 1) * _DH)
    scale = float(_DH) ** -0.5

    pw = cw // ps
    npl = nc * ps

    def piece_rows(slot, isv, c, r):
        cc, j = divmod(c, ps)
        return kvbuf[slot, isv, cc, r * pg:(r + 1) * pg, :, j * pw:(j + 1) * pw].reshape(pr, pw)

    def scores_phase(step, adv):
        g, b, slot = split_step(step)
        sched = _spread(npc * npl, upb - 1)
        qrow = q_scr[g, pl.ds(b, 1), :]
        qbd = jnp.where(diag, jnp.broadcast_to(qrow, (_HG, R)), 0.0).astype(_BF16)
        parts = [None] * npl
        for u in range(upb):
            adv(u)
            for i in sched.get(u, []):
                r, c = divmod(i, npl)
                t = _dot(qbd[:, r * pr:(r + 1) * pr], piece_rows(slot, 0, c, r))
                parts[c] = t if r == 0 else t + parts[c]
        s = jnp.concatenate(parts, axis=-1) * scale
        mx = jnp.max(s, axis=-1, keepdims=True)
        p = jnp.exp(s - mx)
        l = jnp.sum(p, axis=-1, keepdims=True)
        return (p / l).astype(_BF16)

    def values_phase(step, pb, adv, nslots):
        g, b, slot = split_step(step)
        sched = _spread(npc * npl, nslots)
        parts = [None] * npc
        for u in range(nslots):
            adv(u)
            for i in sched.get(u, []):
                r, c = divmod(i, npl)
                t = _dot_nt(pb[:, c * pw:(c + 1) * pw], piece_rows(slot, 1, c, r))
                parts[r] = t if c == 0 else t + parts[r]
        o = jnp.where(diag, jnp.concatenate(parts, axis=-1), 0.0)
        o_scr[pl.ds(b, 1), :] = jnp.sum(o, axis=0, keepdims=True)

    def project(g):
        attn_scr[...] += _dot(o_scr[...].astype(_BF16), wo_buf[pl.ds(g * gpo, gpo)].reshape(R, D))

    def step_body(step, carry):
        def unit(u):
            return kv_unit(step, u) if u < U else kv_unit(step + 1, u - U)

        def adv(u):
            advance(unit(u), P + u, unit(u + dh), unit(u + dl))
        pb = scores_phase(step, lambda u: adv(upb + u))
        values_phase(step, pb, lambda u: adv(U + u), upb)

        @pl.when(lax.rem(step, B) == B - 1)
        def _():
            project(lax.div(step, B))
        return carry

    lax.fori_loop(0, nsteps - 1, step_body, 0)
    last = nsteps - 1
    pb = scores_phase(last, lambda u: advance_static(P + last * U + upb + u))
    base = P + nsteps * U
    values_phase(last, pb, lambda u: advance_static(base + u), len(wo3_u))
    cur = [len(wo3_u)]

    def run_to(mark):
        while cur[0] < mark:
            advance_static(base + cur[0])
            cur[0] += 1

    project(G - 1)
    run_to(cur[0] + wsplit['gap'])

    x = x_buf[...].astype(_F32)
    x1 = x + mod_scr[2] * attn_scr[...]
    h2 = _layernorm(x1) * (1.0 + mod_scr[4]) + mod_scr[3]
    y = _layernorm(h2).astype(_BF16)
    b1 = b1_buf[...].astype(_F32)
    b2 = b2_buf[...].astype(_F32)
    mlp = jnp.concatenate([b2[i:i + 1, :] for i in range(D // _LANE)], axis=-1)
    run_to(len(wo3_u) + len(w1_u))
    hs = []
    tpc = fc // _LANE
    for j in range(nfc):
        b1j = jnp.concatenate([b1[i:i + 1, :] for i in range(j * tpc, (j + 1) * tpc)], axis=-1)
        hs.append(_gelu_tanh(_dot(y, w1_buf[:, :, j * fc:(j + 1) * fc].reshape(D, fc)) + b1j).astype(_BF16))
        run_to(cur[0] + wsplit['gap2'])
    hh = jnp.concatenate(hs, axis=-1)
    done = 0
    for have in wsplit['w2marks']:
        run_to(E - len(w2_u) + have // wsplit['w2'][0])
        mlp = mlp + _dot(hh[:, done:have], w2_buf[0, done:have, :])
        done = have
    out_buf[...] = (x1 + mod_scr[5] * mlp).astype(out_buf.dtype)
    cp_out.start()
    cp_out.wait()


_WSPLIT = dict(wm=(8, 2, 640), wq=(8, 2, 768), wo=(6, 1, 640), wo3=(4, 1, 640, 16), w1=(4, 1, 1536),
               w2=(64, 16), w2marks=(768, 1152, 1408, 1536), gap=4, gap2=3,
               rm=80, rq=80, ro=384, r1=160, r2=1536)


def _run(A_x, A_k_cache, A_v_cache, A_wq, A_wo, B_w1, B_b1, B_w2, B_b2, c, w_mod,
         *, cw=256, m=6, n=16, nh=4, corder=(2, 0, 3, 1), pg=16, ps=1, dl=24, dh=12, ns=24, fc=512, wsplit=None,
         nobc=True, nosc=True):
    B, Sq, D = A_x.shape
    _, Hkv, Sk, Dh = A_k_cache.shape
    F = B_w1.shape[1]
    assert Sq == 1 and Hkv == _HQ and Dh == _DH and B == 8
    W = min(4096, max(256, Sk // 4))
    G = _HQ // _HG
    R = _HG * _DH
    GR = m * _SUB
    ws = dict(_WSPLIT)
    ws.update(wsplit or {})

    x2 = A_x.reshape(B, D)
    kt = jnp.swapaxes(A_k_cache, 2, 3).reshape(B * G, R // GR, GR, Sk)
    vt = jnp.swapaxes(A_v_cache, 2, 3).reshape(B * G, R // GR, GR, Sk)
    wm = w_mod.reshape(-1, ws['rm'], w_mod.shape[1])
    wq = A_wq.reshape(-1, ws['rq'], A_wq.shape[1])
    wo = A_wo.reshape(-1, ws['ro'], D)
    w1 = B_w1.reshape(-1, ws['r1'], F)
    w2 = B_w2.reshape(-1, ws['r2'], D)
    b1 = B_b1.reshape(F // _LANE, _LANE)
    b2 = B_b2.reshape(D // _LANE, _LANE)

    kern = functools.partial(_kernel, B=B, D=D, F=F, Sk=Sk, W=W, cw=cw, m=m, n=n, nh=nh, corder=corder, pg=pg, ps=ps,
                             dl=dl, dh=dh, ns=ns, fc=fc, wsplit=ws)
    any_spec = pl.BlockSpec(memory_space=pl.ANY)
    out = pl.pallas_call(
        kern,
        in_specs=[any_spec] * 11,
        out_specs=any_spec,
        out_shape=jax.ShapeDtypeStruct((B, D), A_x.dtype),
        scratch_shapes=[
            pltpu.VMEM((2, 2, W // cw, R // GR, GR, cw), _BF16),
            pltpu.VMEM(wm.shape, _BF16),
            pltpu.VMEM(wq.shape, _BF16),
            pltpu.VMEM(wo.shape, _BF16),
            pltpu.VMEM(w1.shape, _BF16),
            pltpu.VMEM(w2.shape, _BF16),
            pltpu.VMEM((B, D), _BF16),
            pltpu.VMEM((B, D), _BF16),
            pltpu.VMEM((F // _LANE, _LANE), _BF16),
            pltpu.VMEM((D // _LANE, _LANE), _BF16),
            pltpu.VMEM((B, D), A_x.dtype),
            pltpu.VMEM((6, B, D), _F32),
            pltpu.VMEM((G, B, R), _F32),
            pltpu.VMEM((B, R), _F32),
            pltpu.VMEM((B, D), _F32),
            pltpu.SemaphoreType.DMA((2 * ns + 5,)),
        ],
        compiler_params=pltpu.CompilerParams(vmem_limit_bytes=100 * 1024 * 1024, disable_bounds_checks=nobc,
                                             disable_semaphore_checks=nosc),
    )(x2, kt, vt, wq, wo, w1, b1, w2, b2, c, wm)
    return out.reshape(B, Sq, D)


@jax.jit
def pallas_adaLN_cond__sliding_block_cached__mixer_channel_mlp__decode_kernel(
    A_x: jax.Array,
    A_k_cache: jax.Array,
    A_v_cache: jax.Array,
    A_wq: jax.Array,
    A_wo: jax.Array,
    B_x: jax.Array,
    B_w1: jax.Array,
    B_b1: jax.Array,
    B_w2: jax.Array,
    B_b2: jax.Array,
    c: jax.Array,
    w_mod: jax.Array,
):
    del B_x
    return _run(A_x, A_k_cache, A_v_cache, A_wq, A_wo, B_w1, B_b1, B_w2, B_b2, c, w_mod)
```

```python
import functools

import jax
import jax.numpy as jnp
from jax import lax
import jax.experimental.pallas as pl
import jax.experimental.pallas.tpu as pltpu

_F32 = jnp.float32
_BF16 = jnp.bfloat16

_HQ = 32
_DH = 192
_HG = 8
_LANE = 128
_SUB = 8


def _layernorm(x, eps=1e-5):
    m = jnp.mean(x, axis=-1, keepdims=True)
    xc = x - m
    v = jnp.mean(xc * xc, axis=-1, keepdims=True)
    return xc / jnp.sqrt(v + eps)


def _gelu_tanh(x):
    return 0.5 * x * (1.0 + jnp.tanh(0.7978845608028654 * (x + 0.044715 * (x * x * x))))


def _dot(a, b):
    return jnp.dot(a, b, preferred_element_type=_F32)


def _dot_nt(a, b):
    return lax.dot_general(a, b, (((1,), (1,)), ((), ())), preferred_element_type=_F32)


def _spread(n_items, n_slots, first=0):
    out = {}
    span = n_slots - first
    for i in range(n_items):
        out.setdefault(first + (i * span) // n_items, []).append(i)
    return out


def _kernel(x_hbm, k_hbm, v_hbm, wq_hbm, wo_hbm, w1_hbm, b1_hbm, w2_hbm, b2_hbm, c_hbm, wm_hbm,
            out_hbm,
            kvbuf, wm_buf, wq_buf, wo_buf, w1_buf, w2_buf,
            x_buf, c_buf, b1_buf, b2_buf, out_buf,
            mod_scr, q_scr, o_scr, attn_scr,
            sem,
            *, B, D, F, Sk, W, cw, m, n, nh, corder, pg, ps, gs, hoist, dl, dh, ns, fc, wsplit):
    G = _HQ // _HG
    R = _HG * _DH
    nc = W // cw
    GR = m * _SUB
    NG = R // GR
    rows_u = [(ph, g0) for ph in range(m) for g0 in range(0, NG, n)]
    blk_units = [(r, c) for r in rows_u for c in corder]
    upb = len(blk_units)
    U = 2 * upb
    nsteps = G * B
    nfc = F // fc
    npc = NG // pg
    pr = pg * GR
    assert U % ns == 0 and dl <= ns and dh + hoist <= ns and dl <= upb and dh + hoist <= upb and hoist <= gs

    S_X, S_C, S_B1, S_B2, S_OUT = (2 * ns + i for i in range(5))

    def strided_units(src, dst, g_lo, g_hi, n_, nh_, cw_, rr=_SUB):
        out = []
        for r in range(0, src.shape[1], rr):
            for g0 in range(g_lo, g_hi, n_):
                for c0 in range(0, src.shape[2], cw_):
                    rs, cs = pl.ds(r, rr), pl.ds(c0, cw_)
                    lo, hi = pl.ds(g0, n_ - nh_), pl.ds(g0 + n_ - nh_, nh_)
                    out.append(((src.at[lo, rs, cs], dst.at[lo, rs, cs]),
                                (src.at[hi, rs, cs], dst.at[hi, rs, cs])))
        return out

    def seq_units(src, dst, g, rows, hrows):
        out = []
        for r in range(0, src.shape[1], rows):
            lo, hi = pl.ds(r, rows - hrows), pl.ds(r + rows - hrows, hrows)
            out.append(((src.at[g, lo, :], dst.at[g, lo, :]), (src.at[g, hi, :], dst.at[g, hi, :])))
        return out

    gpo = wo_hbm.shape[0] // G
    wm_u = strided_units(wm_hbm, wm_buf, 0, wm_hbm.shape[0], *wsplit['wm'])
    wq_u = strided_units(wq_hbm, wq_buf, 0, wq_hbm.shape[0], *wsplit['wq'])
    wo_u = strided_units(wo_hbm, wo_buf, 0, (G - 1) * gpo, *wsplit['wo'])
    pro = wm_u + wq_u + wo_u
    P = len(pro)
    wo3_u = strided_units(wo_hbm, wo_buf, (G - 1) * gpo, G * gpo, *wsplit['wo3'])
    w1_u = strided_units(w1_hbm, w1_buf, 0, w1_hbm.shape[0], *wsplit['w1'])
    w2_u = seq_units(w2_hbm, w2_buf, 0, *wsplit['w2'])
    epi = wo3_u + w1_u + w2_u
    E = len(epi)

    def split_step(step):
        if isinstance(step, int):
            return step // B, step % B, step % 2
        return lax.div(step, B), lax.rem(step, B), lax.rem(step, 2)

    def kv_unit(step, u):
        isv, uu = divmod(u, upb)
        (ph, g0), c = blk_units[uu]
        g, b, slot = split_step(step)
        idx = b * G + g
        src = (v_hbm if isv else k_hbm)
        lanes = pl.ds(Sk - W + c * cw, cw)
        rs = pl.ds(ph * _SUB, _SUB)
        lo, hi = pl.ds(g0, n - nh), pl.ds(g0 + n - nh, nh)
        return ((src.at[idx, lo, rs, lanes], kvbuf.at[slot, isv, c, lo, rs, :]),
                (src.at[idx, hi, rs, lanes], kvbuf.at[slot, isv, c, hi, rs, :]))

    def copy(unit, pos, cls):
        s, d = unit[cls]
        return pltpu.make_async_copy(s, d, sem.at[cls * ns + pos % ns])

    def start(unit, pos, cls):
        copy(unit, pos, cls).start(priority=1 - cls)

    def static_unit(pos):
        if pos < P:
            return pro[pos]
        if pos < P + nsteps * U:
            return kv_unit((pos - P) // U, (pos - P) % U)
        if pos < P + nsteps * U + E:
            return epi[pos - P - nsteps * U]
        return None

    def advance(unit, pos, skip_h=False):
        copy(unit(pos), pos, 0).wait()
        copy(unit(pos), pos, 1).wait()
        if not skip_h:
            start_h(unit, pos)
        if unit(pos + dl) is not None:
            start(unit(pos + dl), pos + dl, 0)

    def start_h(unit, pos):
        if unit(pos + dh) is not None:
            start(unit(pos + dh), pos + dh, 1)

    def advance_static(pos):
        advance(static_unit, pos)

    def phase(unit, pos0, nslots, nitems, item):
        sched = _spread(nitems // gs, nslots - hoist)
        hoisted = set()
        for u in range(nslots):
            advance(unit, pos0 + u, skip_h=u in hoisted)
            for gi in sched.get(u, []):
                for j in range(gs):
                    item(gi * gs + j)
                    k = j - (gs - hoist)
                    if k >= 0 and (u + 1 + k) not in hoisted and u + 1 + k < nslots:
                        start_h(unit, pos0 + u + 1 + k)
                        hoisted.add(u + 1 + k)

    cp_x = pltpu.make_async_copy(x_hbm, x_buf, sem.at[S_X])
    cp_c = pltpu.make_async_copy(c_hbm, c_buf, sem.at[S_C])
    cp_b1 = pltpu.make_async_copy(b1_hbm, b1_buf, sem.at[S_B1])
    cp_b2 = pltpu.make_async_copy(b2_hbm, b2_buf, sem.at[S_B2])
    cp_out = pltpu.make_async_copy(out_buf, out_hbm, sem.at[S_OUT])

    for p in range(max(dl, dh)):
        if p < dl:
            start(static_unit(p), p, 0)
        if p < dh:
            start(static_unit(p), p, 1)
    cp_c.start()
    cp_x.start()
    cp_b1.start()
    cp_b2.start()

    pieces = {}

    def at(pos, fn):
        pieces.setdefault(pos, []).append(fn)

    def sc_val():
        c = c_buf[...].astype(_F32)
        return (c * jax.nn.sigmoid(c)).astype(_BF16)

    def wait_small():
        cp_c.wait()
        cp_x.wait()
        cp_b1.wait()
        cp_b2.wait()
        attn_scr[...] = jnp.zeros_like(attn_scr)
    at(len(wm_u) - 2, wait_small)

    def mod_piece(j):
        def f():
            mod_scr[j] = _dot(sc_val(), wm_buf[:, :, j * D:(j + 1) * D].reshape(D, D))
        return f
    for j in range(6):
        at(len(wm_u) - 1 + 4 * j, mod_piece(j))

    def h_piece():
        x = x_buf[...].astype(_F32)
        mod_scr[0] = _layernorm(x) * (1.0 + mod_scr[1]) + mod_scr[0]
    at(len(wm_u) + 24, h_piece)

    qw = 512

    def q_piece(j):
        def f():
            q = _dot(mod_scr[0].astype(_BF16), wq_buf[:, :, j * qw:(j + 1) * qw].reshape(D, qw))
            g, o = divmod(j * qw, R)
            q_scr[g, :, o:o + qw] = q.astype(_BF16).astype(_F32)
        return f
    for j in range(_HQ * _DH // qw):
        at(len(wm_u) + len(wq_u) - 1 + 3 * j, q_piece(j))

    for p in range(P + upb):
        advance_static(p)
        for f in pieces.get(p, []):
            f()

    row = lax.broadcasted_iota(jnp.int32, (_HG, R), 0)
    col = lax.broadcasted_iota(jnp.int32, (_HG, R), 1)
    diag = (col >= row * _DH) & (col < (row + 1) * _DH)
    scale = float(_DH) ** -0.5

    pw = cw // ps
    npl = nc * ps

    def piece_rows(slot, isv, c, r):
        cc, j = divmod(c, ps)
        return kvbuf[slot, isv, cc, r * pg:(r + 1) * pg, :, j * pw:(j + 1) * pw].reshape(pr, pw)

    def scores_phase(step, unit, pos0):
        g, b, slot = split_step(step)
        qrow = q_scr[g, pl.ds(b, 1), :]
        qbd = jnp.where(diag, jnp.broadcast_to(qrow, (_HG, R)), 0.0).astype(_BF16)
        parts = [None] * npl

        def item(i):
            r, c = divmod(i, npl)
            t = _dot(qbd[:, r * pr:(r + 1) * pr], piece_rows(slot, 0, c, r))
            parts[c] = t if r == 0 else t + parts[c]
        phase(unit, pos0, upb, npc * npl, item)
        s = jnp.concatenate(parts, axis=-1) * scale
        mx = jnp.max(s, axis=-1, keepdims=True)
        p = jnp.exp(s - mx)
        l = jnp.sum(p, axis=-1, keepdims=True)
        return (p / l).astype(_BF16)

    def values_phase(step, pb, unit, pos0, nslots):
        g, b, slot = split_step(step)
        parts = [None] * npc

        def item(i):
            r, c = divmod(i, npl)
            t = _dot_nt(pb[:, c * pw:(c + 1) * pw], piece_rows(slot, 1, c, r))
            parts[r] = t if c == 0 else t + parts[r]
        phase(unit, pos0, nslots, npc * npl, item)
        o = jnp.where(diag, jnp.concatenate(parts, axis=-1), 0.0)
        o_scr[pl.ds(b, 1), :] = jnp.sum(o, axis=0, keepdims=True)

    def project(g):
        attn_scr[...] += _dot(o_scr[...].astype(_BF16), wo_buf[pl.ds(g * gpo, gpo)].reshape(R, D))

    def step_body(step, carry):
        def unit(pos):
            u = pos - P
            return kv_unit(step, u) if u < U else kv_unit(step + 1, u - U)
        pb = scores_phase(step, unit, P + upb)
        values_phase(step, pb, unit, P + U, upb)

        @pl.when(lax.rem(step, B) == B - 1)
        def _():
            project(lax.div(step, B))
        return carry

    lax.fori_loop(0, nsteps - 1, step_body, 0)
    last = nsteps - 1
    pb = scores_phase(last, static_unit, P + last * U + upb)
    base = P + nsteps * U
    values_phase(last, pb, static_unit, base, len(wo3_u))
    cur = [len(wo3_u)]

    def run_to(mark):
        while cur[0] < mark:
            advance_static(base + cur[0])
            cur[0] += 1

    project(G - 1)
    run_to(cur[0] + wsplit['gap'])

    x = x_buf[...].astype(_F32)
    x1 = x + mod_scr[2] * attn_scr[...]
    h2 = _layernorm(x1) * (1.0 + mod_scr[4]) + mod_scr[3]
    y = _layernorm(h2).astype(_BF16)
    b1 = b1_buf[...].astype(_F32)
    b2 = b2_buf[...].astype(_F32)
    mlp = jnp.concatenate([b2[i:i + 1, :] for i in range(D // _LANE)], axis=-1)
    run_to(len(wo3_u) + len(w1_u))
    hs = []
    tpc = fc // _LANE
    for j in range(nfc):
        b1j = jnp.concatenate([b1[i:i + 1, :] for i in range(j * tpc, (j + 1) * tpc)], axis=-1)
        hs.append(_gelu_tanh(_dot(y, w1_buf[:, :, j * fc:(j + 1) * fc].reshape(D, fc)) + b1j).astype(_BF16))
        run_to(cur[0] + wsplit['gap2'])
    hh = jnp.concatenate(hs, axis=-1)
    done = 0
    for have in wsplit['w2marks']:
        run_to(E - len(w2_u) + have // wsplit['w2'][0])
        mlp = mlp + _dot(hh[:, done:have], w2_buf[0, done:have, :])
        done = have
    out_buf[...] = (x1 + mod_scr[5] * mlp).astype(out_buf.dtype)
    cp_out.start()
    cp_out.wait()


_WSPLIT = dict(wm=(8, 2, 640), wq=(8, 2, 768), wo=(6, 1, 640), wo3=(4, 1, 640, 16), w1=(4, 1, 1536),
               w2=(64, 16), w2marks=(768, 1152, 1408, 1536), gap=4, gap2=3,
               rm=80, rq=80, ro=384, r1=160, r2=1536)


def _run(A_x, A_k_cache, A_v_cache, A_wq, A_wo, B_w1, B_b1, B_w2, B_b2, c, w_mod,
         *, cw=256, m=6, n=16, nh=4, corder=(2, 0, 3, 1), pg=16, ps=1, gs=2, hoist=2, dl=24, dh=12, ns=24, fc=512, wsplit=None,
         nobc=True, nosc=True):
    B, Sq, D = A_x.shape
    _, Hkv, Sk, Dh = A_k_cache.shape
    F = B_w1.shape[1]
    assert Sq == 1 and Hkv == _HQ and Dh == _DH and B == 8
    W = min(4096, max(256, Sk // 4))
    G = _HQ // _HG
    R = _HG * _DH
    GR = m * _SUB
    ws = dict(_WSPLIT)
    ws.update(wsplit or {})

    x2 = A_x.reshape(B, D)
    kt = jnp.swapaxes(A_k_cache, 2, 3).reshape(B * G, R // GR, GR, Sk)
    vt = jnp.swapaxes(A_v_cache, 2, 3).reshape(B * G, R // GR, GR, Sk)
    wm = w_mod.reshape(-1, ws['rm'], w_mod.shape[1])
    wq = A_wq.reshape(-1, ws['rq'], A_wq.shape[1])
    wo = A_wo.reshape(-1, ws['ro'], D)
    w1 = B_w1.reshape(-1, ws['r1'], F)
    w2 = B_w2.reshape(-1, ws['r2'], D)
    b1 = B_b1.reshape(F // _LANE, _LANE)
    b2 = B_b2.reshape(D // _LANE, _LANE)

    kern = functools.partial(_kernel, B=B, D=D, F=F, Sk=Sk, W=W, cw=cw, m=m, n=n, nh=nh, corder=corder, pg=pg, ps=ps, gs=gs, hoist=hoist,
                             dl=dl, dh=dh, ns=ns, fc=fc, wsplit=ws)
    any_spec = pl.BlockSpec(memory_space=pl.ANY)
    out = pl.pallas_call(
        kern,
        in_specs=[any_spec] * 11,
        out_specs=any_spec,
        out_shape=jax.ShapeDtypeStruct((B, D), A_x.dtype),
        scratch_shapes=[
            pltpu.VMEM((2, 2, W // cw, R // GR, GR, cw), _BF16),
            pltpu.VMEM(wm.shape, _BF16),
            pltpu.VMEM(wq.shape, _BF16),
            pltpu.VMEM(wo.shape, _BF16),
            pltpu.VMEM(w1.shape, _BF16),
            pltpu.VMEM(w2.shape, _BF16),
            pltpu.VMEM((B, D), _BF16),
            pltpu.VMEM((B, D), _BF16),
            pltpu.VMEM((F // _LANE, _LANE), _BF16),
            pltpu.VMEM((D // _LANE, _LANE), _BF16),
            pltpu.VMEM((B, D), A_x.dtype),
            pltpu.VMEM((6, B, D), _F32),
            pltpu.VMEM((G, B, R), _F32),
            pltpu.VMEM((B, R), _F32),
            pltpu.VMEM((B, D), _F32),
            pltpu.SemaphoreType.DMA((2 * ns + 5,)),
        ],
        compiler_params=pltpu.CompilerParams(vmem_limit_bytes=100 * 1024 * 1024, disable_bounds_checks=nobc,
                                             disable_semaphore_checks=nosc),
    )(x2, kt, vt, wq, wo, w1, b1, w2, b2, c, wm)
    return out.reshape(B, Sq, D)


@jax.jit
def pallas_adaLN_cond__sliding_block_cached__mixer_channel_mlp__decode_kernel(
    A_x: jax.Array,
    A_k_cache: jax.Array,
    A_v_cache: jax.Array,
    A_wq: jax.Array,
    A_wo: jax.Array,
    B_x: jax.Array,
    B_w1: jax.Array,
    B_b1: jax.Array,
    B_w2: jax.Array,
    B_b2: jax.Array,
    c: jax.Array,
    w_mod: jax.Array,
):
    del B_x
    return _run(A_x, A_k_cache, A_v_cache, A_wq, A_wo, B_w1, B_b1, B_w2, B_b2, c, w_mod)
```

```python
import functools

import jax
import jax.numpy as jnp
from jax import lax
import jax.experimental.pallas as pl
import jax.experimental.pallas.tpu as pltpu

_F32 = jnp.float32
_BF16 = jnp.bfloat16

_HQ = 32
_DH = 192
_HG = 8
_LANE = 128
_SUB = 8

_CW = 256
_CORDER = (2, 0, 3, 1)
_KV_STRIDE = 6
_KV_N, _KV_NH = 16, 4
_DL, _DH_AHEAD, _NS = 24, 12, 24
_RM, _RQ, _RO, _R1 = 80, 80, 384, 160
_U_WM, _U_WQ, _U_WO = (8, 2, 640, 8), (8, 2, 768, 8), (6, 1, 640, 8)
_U_WO_LAST, _U_W1 = (4, 1, 640, 16), (4, 1, 1536, 8)
_U_W2 = (64, 16)
_W2_MARKS = (768, 1152, 1408, 1536)
_PG = 16
_GS = 2
_QW = 512
_FC = 512


def _layernorm(x, eps=1e-5):
    m = jnp.mean(x, axis=-1, keepdims=True)
    xc = x - m
    v = jnp.mean(xc * xc, axis=-1, keepdims=True)
    return xc / jnp.sqrt(v + eps)


def _gelu_tanh(x):
    return 0.5 * x * (1.0 + jnp.tanh(0.7978845608028654 * (x + 0.044715 * (x * x * x))))


def _dot(a, b):
    return jnp.dot(a, b, preferred_element_type=_F32)


def _dot_nt(a, b):
    return lax.dot_general(a, b, (((1,), (1,)), ((), ())), preferred_element_type=_F32)


def _row_vector(tiles, lo, hi):
    return jnp.concatenate([tiles[i:i + 1, :] for i in range(lo, hi)], axis=-1)


def _kernel(x_hbm, k_hbm, v_hbm, wq_hbm, wo_hbm, w1_hbm, b1_hbm, w2_hbm, b2_hbm, c_hbm, wm_hbm,
            out_hbm,
            kvbuf, wm_buf, wq_buf, wo_buf, w1_buf, w2_buf,
            x_buf, c_buf, b1_buf, b2_buf, out_buf,
            mod_scr, q_scr, o_scr, attn_scr,
            sem,
            *, B, D, F, Sk, W):
    G = _HQ // _HG
    R = _HG * _DH
    nc = W // _CW
    GR = _KV_STRIDE * _SUB
    NG = R // GR
    blk_units = [(ph, g0, c) for ph in range(_KV_STRIDE) for g0 in range(0, NG, _KV_N) for c in _CORDER]
    upb = len(blk_units)
    U = 2 * upb
    nsteps = G * B
    npc = NG // _PG
    pr = _PG * GR
    assert sorted(_CORDER) == list(range(nc))
    assert U % _NS == 0 and _DL <= min(_NS, upb) and _DH_AHEAD + _GS <= min(_NS, upb)

    def strided_units(src, dst, g_lo, g_hi, n, nh, cw, rr):
        out = []
        for r in range(0, src.shape[1], rr):
            for g0 in range(g_lo, g_hi, n):
                for c0 in range(0, src.shape[2], cw):
                    rs, cs = pl.ds(r, rr), pl.ds(c0, cw)
                    lo, hi = pl.ds(g0, n - nh), pl.ds(g0 + n - nh, nh)
                    out.append(((src.at[lo, rs, cs], dst.at[lo, rs, cs]),
                                (src.at[hi, rs, cs], dst.at[hi, rs, cs])))
        return out

    def sequential_units(src, dst, rows, hrows):
        out = []
        for r in range(0, src.shape[0], rows):
            lo, hi = pl.ds(r, rows - hrows), pl.ds(r + rows - hrows, hrows)
            out.append(((src.at[lo, :], dst.at[lo, :]), (src.at[hi, :], dst.at[hi, :])))
        return out

    gpo = wo_hbm.shape[0] // G
    wm_u = strided_units(wm_hbm, wm_buf, 0, wm_hbm.shape[0], *_U_WM)
    wq_u = strided_units(wq_hbm, wq_buf, 0, wq_hbm.shape[0], *_U_WQ)
    wo_u = strided_units(wo_hbm, wo_buf, 0, (G - 1) * gpo, *_U_WO)
    head = wm_u + wq_u + wo_u
    wo_last_u = strided_units(wo_hbm, wo_buf, (G - 1) * gpo, G * gpo, *_U_WO_LAST)
    w1_u = strided_units(w1_hbm, w1_buf, 0, w1_hbm.shape[0], *_U_W1)
    w2_u = sequential_units(w2_hbm, w2_buf, *_U_W2)
    tail = wo_last_u + w1_u + w2_u
    P, E = len(head), len(tail)

    def split_step(step):
        if isinstance(step, int):
            return step // B, step % B, step % 2
        return lax.div(step, B), lax.rem(step, B), lax.rem(step, 2)

    def kv_unit(step, u):
        isv, uu = divmod(u, upb)
        ph, g0, c = blk_units[uu]
        g, b, slot = split_step(step)
        idx = b * G + g
        src = v_hbm if isv else k_hbm
        lanes = pl.ds(Sk - W + c * _CW, _CW)
        rs = pl.ds(ph * _SUB, _SUB)
        lo, hi = pl.ds(g0, _KV_N - _KV_NH), pl.ds(g0 + _KV_N - _KV_NH, _KV_NH)
        return ((src.at[idx, lo, rs, lanes], kvbuf.at[slot, isv, c, lo, rs, :]),
                (src.at[idx, hi, rs, lanes], kvbuf.at[slot, isv, c, hi, rs, :]))

    def static_unit(pos):
        if pos < P:
            return head[pos]
        if pos < P + nsteps * U:
            return kv_unit((pos - P) // U, (pos - P) % U)
        if pos < P + nsteps * U + E:
            return tail[pos - P - nsteps * U]
        return None

    def copy(unit, pos, cls):
        s, d = unit(pos)[cls]
        return pltpu.make_async_copy(s, d, sem.at[cls * _NS + pos % _NS])

    def start(unit, pos, cls):
        if unit(pos) is not None:
            copy(unit, pos, cls).start(priority=1 - cls)

    def advance(unit, pos, skip_high=False):
        copy(unit, pos, 0).wait()
        copy(unit, pos, 1).wait()
        if not skip_high:
            start(unit, pos + _DH_AHEAD, 1)
        start(unit, pos + _DL, 0)

    def phase(unit, pos0, nslots, nitems, item):
        nbursts = nitems // _GS
        at = {(i * (nslots - _GS)) // nbursts: i for i in range(nbursts)}
        assert len(at) == nbursts
        early = set()
        for u in range(nslots):
            advance(unit, pos0 + u, skip_high=u in early)
            if u in at:
                for j in range(_GS):
                    item(at[u] * _GS + j)
                    if u + 1 + j not in early:
                        start(unit, pos0 + u + 1 + j + _DH_AHEAD, 1)
                        early.add(u + 1 + j)

    small = [pltpu.make_async_copy(s, d, sem.at[2 * _NS + i]) for i, (s, d) in enumerate(
        [(c_hbm, c_buf), (x_hbm, x_buf), (b1_hbm, b1_buf), (b2_hbm, b2_buf)])]
    cp_out = pltpu.make_async_copy(out_buf, out_hbm, sem.at[2 * _NS + len(small)])

    for p in range(_DL):
        start(static_unit, p, 0)
        if p < _DH_AHEAD:
            start(static_unit, p, 1)
    for cp in small:
        cp.start()

    def wait_small():
        for cp in small:
            cp.wait()
        attn_scr[...] = jnp.zeros_like(attn_scr)

    def mod_piece(j):
        c = c_buf[...].astype(_F32)
        silu_c = (c * jax.nn.sigmoid(c)).astype(_BF16)
        mod_scr[j] = _dot(silu_c, wm_buf[:, :, j * D:(j + 1) * D].reshape(D, D))

    def h_piece():
        mod_scr[0] = _layernorm(x_buf[...].astype(_F32)) * (1.0 + mod_scr[1]) + mod_scr[0]

    def q_piece(j):
        q = _dot(mod_scr[0].astype(_BF16), wq_buf[:, :, j * _QW:(j + 1) * _QW].reshape(D, _QW))
        g, o = divmod(j * _QW, R)
        q_scr[g, :, o:o + _QW] = q.astype(_BF16).astype(_F32)

    after = {len(wm_u) - 2: wait_small, len(wm_u) + 24: h_piece}
    for j in range(6):
        after[len(wm_u) - 1 + 4 * j] = functools.partial(mod_piece, j)
    for j in range(_HQ * _DH // _QW):
        after[len(wm_u) + len(wq_u) - 1 + 3 * j] = functools.partial(q_piece, j)
    assert len(after) == 8 + _HQ * _DH // _QW and max(after) < P + upb
    for p in range(P + upb):
        advance(static_unit, p)
        if p in after:
            after[p]()

    row = lax.broadcasted_iota(jnp.int32, (_HG, R), 0)
    col = lax.broadcasted_iota(jnp.int32, (_HG, R), 1)
    diag = (col >= row * _DH) & (col < (row + 1) * _DH)
    scale = float(_DH) ** -0.5

    def kv_piece(slot, isv, c, r):
        return kvbuf[slot, isv, c, r * _PG:(r + 1) * _PG].reshape(pr, _CW)

    def scores_phase(step, unit, pos0):
        g, b, slot = split_step(step)
        qrow = q_scr[g, pl.ds(b, 1), :]
        qbd = jnp.where(diag, jnp.broadcast_to(qrow, (_HG, R)), 0.0).astype(_BF16)
        parts = [None] * nc

        def item(i):
            r, c = divmod(i, nc)
            t = _dot(qbd[:, r * pr:(r + 1) * pr], kv_piece(slot, 0, c, r))
            parts[c] = t if r == 0 else t + parts[c]
        phase(unit, pos0, upb, npc * nc, item)
        s = jnp.concatenate(parts, axis=-1) * scale
        p = jnp.exp(s - jnp.max(s, axis=-1, keepdims=True))
        return (p / jnp.sum(p, axis=-1, keepdims=True)).astype(_BF16)

    def values_phase(step, pb, unit, pos0, nslots):
        _, b, slot = split_step(step)
        parts = [None] * npc

        def item(i):
            r, c = divmod(i, nc)
            t = _dot_nt(pb[:, c * _CW:(c + 1) * _CW], kv_piece(slot, 1, c, r))
            parts[r] = t if c == 0 else t + parts[r]
        phase(unit, pos0, nslots, npc * nc, item)
        o = jnp.where(diag, jnp.concatenate(parts, axis=-1), 0.0)
        o_scr[pl.ds(b, 1), :] = jnp.sum(o, axis=0, keepdims=True)

    def project(g):
        attn_scr[...] += _dot(o_scr[...].astype(_BF16), wo_buf[pl.ds(g * gpo, gpo)].reshape(R, D))

    def step_body(step, carry):
        def unit(pos):
            u = pos - P
            return kv_unit(step, u) if u < U else kv_unit(step + 1, u - U)
        pb = scores_phase(step, unit, P + upb)
        values_phase(step, pb, unit, P + U, upb)

        @pl.when(lax.rem(step, B) == B - 1)
        def _():
            project(lax.div(step, B))
        return carry

    lax.fori_loop(0, nsteps - 1, step_body, 0)
    last = nsteps - 1
    base = P + nsteps * U
    pb = scores_phase(last, static_unit, base - upb)
    values_phase(last, pb, static_unit, base, len(wo_last_u))

    cur = [len(wo_last_u)]

    def run_to(mark):
        while cur[0] < mark:
            advance(static_unit, base + cur[0])
            cur[0] += 1

    project(G - 1)
    run_to(cur[0] + 4)
    x1 = x_buf[...].astype(_F32) + mod_scr[2] * attn_scr[...]
    h2 = _layernorm(x1) * (1.0 + mod_scr[4]) + mod_scr[3]
    y = _layernorm(h2).astype(_BF16)
    b1 = b1_buf[...].astype(_F32)
    mlp = _row_vector(b2_buf[...].astype(_F32), 0, D // _LANE)
    run_to(len(wo_last_u) + len(w1_u))
    hs = []
    tpc = _FC // _LANE
    for j in range(F // _FC):
        pre = _dot(y, w1_buf[:, :, j * _FC:(j + 1) * _FC].reshape(D, _FC))
        hs.append(_gelu_tanh(pre + _row_vector(b1, j * tpc, (j + 1) * tpc)).astype(_BF16))
        run_to(cur[0] + 3)
    hh = jnp.concatenate(hs, axis=-1)
    assert _W2_MARKS[-1] == F
    for lo, hi in zip((0,) + _W2_MARKS[:-1], _W2_MARKS):
        run_to(E - len(w2_u) + hi // _U_W2[0])
        mlp = _dot(hh[:, lo:hi], w2_buf[lo:hi, :]) + mlp
    out_buf[...] = (x1 + mod_scr[5] * mlp).astype(out_buf.dtype)
    cp_out.start()
    cp_out.wait()


def _compiler_params():
    base = dict(vmem_limit_bytes=100 * 1024 * 1024)
    try:
        return pltpu.CompilerParams(disable_bounds_checks=True, disable_semaphore_checks=True, **base)
    except TypeError:
        return pltpu.CompilerParams(**base)


def _run(A_x, A_k_cache, A_v_cache, A_wq, A_wo, B_w1, B_b1, B_w2, B_b2, c, w_mod):
    B, Sq, D = A_x.shape
    _, Hkv, Sk, Dh = A_k_cache.shape
    F = B_w1.shape[1]
    assert Sq == 1 and Hkv == _HQ and Dh == _DH and B == _SUB
    W = min(4096, max(256, Sk // 4))
    G = _HQ // _HG
    R = _HG * _DH
    GR = _KV_STRIDE * _SUB

    x2 = A_x.reshape(B, D)
    kt = jnp.swapaxes(A_k_cache, 2, 3).reshape(B * G, R // GR, GR, Sk)
    vt = jnp.swapaxes(A_v_cache, 2, 3).reshape(B * G, R // GR, GR, Sk)
    wm = w_mod.reshape(-1, _RM, w_mod.shape[1])
    wq = A_wq.reshape(-1, _RQ, A_wq.shape[1])
    wo = A_wo.reshape(-1, _RO, D)
    w1 = B_w1.reshape(-1, _R1, F)
    b1 = B_b1.reshape(F // _LANE, _LANE)
    b2 = B_b2.reshape(D // _LANE, _LANE)

    any_spec = pl.BlockSpec(memory_space=pl.ANY)
    out = pl.pallas_call(
        functools.partial(_kernel, B=B, D=D, F=F, Sk=Sk, W=W),
        in_specs=[any_spec] * 11,
        out_specs=any_spec,
        out_shape=jax.ShapeDtypeStruct((B, D), A_x.dtype),
        scratch_shapes=[
            pltpu.VMEM((2, 2, W // _CW, R // GR, GR, _CW), _BF16),
            pltpu.VMEM(wm.shape, _BF16),
            pltpu.VMEM(wq.shape, _BF16),
            pltpu.VMEM(wo.shape, _BF16),
            pltpu.VMEM(w1.shape, _BF16),
            pltpu.VMEM(B_w2.shape, _BF16),
            pltpu.VMEM(x2.shape, _BF16),
            pltpu.VMEM(c.shape, _BF16),
            pltpu.VMEM(b1.shape, _BF16),
            pltpu.VMEM(b2.shape, _BF16),
            pltpu.VMEM((B, D), A_x.dtype),
            pltpu.VMEM((6, B, D), _F32),
            pltpu.VMEM((G, B, R), _F32),
            pltpu.VMEM((B, R), _F32),
            pltpu.VMEM((B, D), _F32),
            pltpu.SemaphoreType.DMA((2 * _NS + 5,)),
        ],
        compiler_params=_compiler_params(),
    )(x2, kt, vt, wq, wo, w1, b1, B_w2, b2, c, wm)
    return out.reshape(B, Sq, D)


@jax.jit
def pallas_adaLN_cond__sliding_block_cached__mixer_channel_mlp__decode_kernel(
    A_x: jax.Array,
    A_k_cache: jax.Array,
    A_v_cache: jax.Array,
    A_wq: jax.Array,
    A_wo: jax.Array,
    B_x: jax.Array,
    B_w1: jax.Array,
    B_b1: jax.Array,
    B_w2: jax.Array,
    B_b2: jax.Array,
    c: jax.Array,
    w_mod: jax.Array,
):
    del B_x
    return _run(A_x, A_k_cache, A_v_cache, A_wq, A_wo, B_w1, B_b1, B_w2, B_b2, c, w_mod)
```

```python
import functools

import jax
import jax.numpy as jnp
from jax import lax
import jax.experimental.pallas as pl
import jax.experimental.pallas.tpu as pltpu

_F32 = jnp.float32
_BF16 = jnp.bfloat16

_HQ = 32
_DH = 192
_HG = 8
_LANE = 128
_SUB = 8

_CW = 256
_CORDER = (2, 0, 3, 1)
_KV_STRIDE = 6
_KV_N, _KV_NH = 16, 4
_DL, _DH_AHEAD, _NS = 24, 12, 24
_RM, _RQ, _RO, _R1 = 80, 80, 384, 160
_U_WM, _U_WQ, _U_WO = (8, 2, 384, 8), (8, 2, 768, 8), (6, 1, 640, 8)
_U_WO_LAST, _U_W1 = (4, 1, 640, 16), (4, 1, 1536, 8)
_WO_LAST_SPAN = 0.73
_U_W2 = (64, 16)
_W2_MARKS = (768, 1152, 1408, 1536)
_PG = 16
_GS = 2
_QW = 512
_FC = 512


def _layernorm(x, eps=1e-5):
    m = jnp.mean(x, axis=-1, keepdims=True)
    xc = x - m
    v = jnp.mean(xc * xc, axis=-1, keepdims=True)
    return xc / jnp.sqrt(v + eps)


def _gelu_tanh(x):
    return 0.5 * x * (1.0 + jnp.tanh(0.7978845608028654 * (x + 0.044715 * (x * x * x))))


def _dot(a, b):
    return jnp.dot(a, b, preferred_element_type=_F32)


def _dot_nt(a, b):
    return lax.dot_general(a, b, (((1,), (1,)), ((), ())), preferred_element_type=_F32)


def _row_vector(tiles, lo, hi):
    return jnp.concatenate([tiles[i:i + 1, :] for i in range(lo, hi)], axis=-1)


def _kernel(x_hbm, k_hbm, v_hbm, wq_hbm, wo_hbm, w1_hbm, b1_hbm, w2_hbm, b2_hbm, c_hbm, wm_hbm,
            out_hbm,
            kvbuf, wm_buf, wq_buf, wo_buf, w1_buf, w2_buf,
            x_buf, c_buf, b1_buf, b2_buf, out_buf,
            mod_scr, q_scr, o_scr, attn_scr,
            sem,
            *, B, D, F, Sk, W):
    G = _HQ // _HG
    R = _HG * _DH
    nc = W // _CW
    GR = _KV_STRIDE * _SUB
    NG = R // GR
    blk_units = [(ph, g0, c) for ph in range(_KV_STRIDE) for g0 in range(0, NG, _KV_N) for c in _CORDER]
    upb = len(blk_units)
    U = 2 * upb
    nsteps = G * B
    npc = NG // _PG
    pr = _PG * GR
    assert sorted(_CORDER) == list(range(nc))
    assert U % _NS == 0 and _DL <= min(_NS, upb) and _DH_AHEAD + _GS <= min(_NS, upb)

    def strided_units(src, dst, g_lo, g_hi, n, nh, cw, rr):
        out = []
        for r in range(0, src.shape[1], rr):
            for g0 in range(g_lo, g_hi, n):
                for c0 in range(0, src.shape[2], cw):
                    rs, cs = pl.ds(r, rr), pl.ds(c0, cw)
                    lo, hi = pl.ds(g0, n - nh), pl.ds(g0 + n - nh, nh)
                    out.append(((src.at[lo, rs, cs], dst.at[lo, rs, cs]),
                                (src.at[hi, rs, cs], dst.at[hi, rs, cs])))
        return out

    def sequential_units(src, dst, rows, hrows):
        out = []
        for r in range(0, src.shape[0], rows):
            lo, hi = pl.ds(r, rows - hrows), pl.ds(r + rows - hrows, hrows)
            out.append(((src.at[lo, :], dst.at[lo, :]), (src.at[hi, :], dst.at[hi, :])))
        return out

    gpo = wo_hbm.shape[0] // G
    wm_u = strided_units(wm_hbm, wm_buf, 0, wm_hbm.shape[0], *_U_WM)
    wq_u = strided_units(wq_hbm, wq_buf, 0, wq_hbm.shape[0], *_U_WQ)
    wo_u = strided_units(wo_hbm, wo_buf, 0, (G - 1) * gpo, *_U_WO)
    head = wm_u + wq_u + wo_u
    wo_last_u = strided_units(wo_hbm, wo_buf, (G - 1) * gpo, G * gpo, *_U_WO_LAST)
    w1_u = strided_units(w1_hbm, w1_buf, 0, w1_hbm.shape[0], *_U_W1)
    w2_u = sequential_units(w2_hbm, w2_buf, *_U_W2)
    mixed = sorted([(_WO_LAST_SPAN * (i + 1) / len(wo_last_u), 0, i) for i in range(len(wo_last_u))]
                   + [((i + 1) / len(w1_u), 1, i) for i in range(len(w1_u))])
    tail = [(wo_last_u, w1_u)[a][i] for _, a, i in mixed] + w2_u
    wo_done = 1 + max(p for p, (_, a, _) in enumerate(mixed) if a == 0)
    w1_done = len(mixed)
    P, E = len(head), len(tail)

    def split_step(step):
        if isinstance(step, int):
            return step // B, step % B, step % 2
        return lax.div(step, B), lax.rem(step, B), lax.rem(step, 2)

    def kv_unit(step, u):
        isv, uu = divmod(u, upb)
        ph, g0, c = blk_units[uu]
        g, b, slot = split_step(step)
        idx = b * G + g
        src = v_hbm if isv else k_hbm
        lanes = pl.ds(Sk - W + c * _CW, _CW)
        rs = pl.ds(ph * _SUB, _SUB)
        lo, hi = pl.ds(g0, _KV_N - _KV_NH), pl.ds(g0 + _KV_N - _KV_NH, _KV_NH)
        return ((src.at[idx, lo, rs, lanes], kvbuf.at[slot, isv, c, lo, rs, :]),
                (src.at[idx, hi, rs, lanes], kvbuf.at[slot, isv, c, hi, rs, :]))

    def static_unit(pos):
        if pos < P:
            return head[pos]
        if pos < P + nsteps * U:
            return kv_unit((pos - P) // U, (pos - P) % U)
        if pos < P + nsteps * U + E:
            return tail[pos - P - nsteps * U]
        return None

    def copy(unit, pos, cls):
        s, d = unit(pos)[cls]
        return pltpu.make_async_copy(s, d, sem.at[cls * _NS + pos % _NS])

    def start(unit, pos, cls):
        if unit(pos) is not None:
            copy(unit, pos, cls).start(priority=1 - cls)

    def advance(unit, pos, skip_high=False):
        copy(unit, pos, 0).wait()
        copy(unit, pos, 1).wait()
        if not skip_high:
            start(unit, pos + _DH_AHEAD, 1)
        start(unit, pos + _DL, 0)

    def phase(unit, pos0, nslots, nitems, item):
        nbursts = nitems // _GS
        at = {(i * (nslots - _GS)) // nbursts: i for i in range(nbursts)}
        assert len(at) == nbursts
        early = set()
        for u in range(nslots):
            advance(unit, pos0 + u, skip_high=u in early)
            if u in at:
                for j in range(_GS):
                    item(at[u] * _GS + j)
                    if u + 1 + j not in early:
                        start(unit, pos0 + u + 1 + j + _DH_AHEAD, 1)
                        early.add(u + 1 + j)

    small = [pltpu.make_async_copy(s, d, sem.at[2 * _NS + i]) for i, (s, d) in enumerate(
        [(c_hbm, c_buf), (x_hbm, x_buf), (b1_hbm, b1_buf), (b2_hbm, b2_buf)])]
    cp_out = pltpu.make_async_copy(out_buf, out_hbm, sem.at[2 * _NS + len(small)])

    for p in range(_DL):
        start(static_unit, p, 0)
        if p < _DH_AHEAD:
            start(static_unit, p, 1)
    for cp in small:
        cp.start()

    def wait_small():
        for cp in small:
            cp.wait()
        attn_scr[...] = jnp.zeros_like(attn_scr)

    def mod_piece(j):
        c = c_buf[...].astype(_F32)
        silu_c = (c * jax.nn.sigmoid(c)).astype(_BF16)
        mod_scr[j] = _dot(silu_c, wm_buf[:, :, j * D:(j + 1) * D].reshape(D, D))

    def h_piece():
        mod_scr[0] = _layernorm(x_buf[...].astype(_F32)) * (1.0 + mod_scr[1]) + mod_scr[0]

    def q_piece(j):
        q = _dot(mod_scr[0].astype(_BF16), wq_buf[:, :, j * _QW:(j + 1) * _QW].reshape(D, _QW))
        g, o = divmod(j * _QW, R)
        q_scr[g, :, o:o + _QW] = q.astype(_BF16).astype(_F32)

    after = {len(wm_u) - 2: wait_small, len(wm_u) + 24: h_piece}
    for j in range(6):
        after[len(wm_u) - 1 + 4 * j] = functools.partial(mod_piece, j)
    for j in range(_HQ * _DH // _QW):
        after[len(wm_u) + len(wq_u) - 1 + 3 * j] = functools.partial(q_piece, j)
    assert len(after) == 8 + _HQ * _DH // _QW and max(after) < P + upb
    for p in range(P + upb):
        advance(static_unit, p)
        if p in after:
            after[p]()

    row = lax.broadcasted_iota(jnp.int32, (_HG, R), 0)
    col = lax.broadcasted_iota(jnp.int32, (_HG, R), 1)
    diag = (col >= row * _DH) & (col < (row + 1) * _DH)
    scale = float(_DH) ** -0.5

    def kv_piece(slot, isv, c, r):
        return kvbuf[slot, isv, c, r * _PG:(r + 1) * _PG].reshape(pr, _CW)

    def scores_phase(step, unit, pos0):
        g, b, slot = split_step(step)
        qrow = q_scr[g, pl.ds(b, 1), :]
        qbd = jnp.where(diag, jnp.broadcast_to(qrow, (_HG, R)), 0.0).astype(_BF16)
        parts = [None] * nc

        def item(i):
            r, c = divmod(i, nc)
            t = _dot(qbd[:, r * pr:(r + 1) * pr], kv_piece(slot, 0, c, r))
            parts[c] = t if r == 0 else t + parts[c]
        phase(unit, pos0, upb, npc * nc, item)
        s = jnp.concatenate(parts, axis=-1) * scale
        p = jnp.exp(s - jnp.max(s, axis=-1, keepdims=True))
        return (p / jnp.sum(p, axis=-1, keepdims=True)).astype(_BF16)

    def values_phase(step, pb, unit, pos0, nslots):
        _, b, slot = split_step(step)
        parts = [None] * npc

        def item(i):
            r, c = divmod(i, nc)
            t = _dot_nt(pb[:, c * _CW:(c + 1) * _CW], kv_piece(slot, 1, c, r))
            parts[r] = t if c == 0 else t + parts[r]
        phase(unit, pos0, nslots, npc * nc, item)
        o = jnp.where(diag, jnp.concatenate(parts, axis=-1), 0.0)
        o_scr[pl.ds(b, 1), :] = jnp.sum(o, axis=0, keepdims=True)

    def project(g):
        attn_scr[...] += _dot(o_scr[...].astype(_BF16), wo_buf[pl.ds(g * gpo, gpo)].reshape(R, D))

    def step_body(step, carry):
        def unit(pos):
            u = pos - P
            return kv_unit(step, u) if u < U else kv_unit(step + 1, u - U)
        pb = scores_phase(step, unit, P + upb)
        values_phase(step, pb, unit, P + U, upb)

        @pl.when(lax.rem(step, B) == B - 1)
        def _():
            project(lax.div(step, B))
        return carry

    lax.fori_loop(0, nsteps - 1, step_body, 0)
    last = nsteps - 1
    base = P + nsteps * U
    pb = scores_phase(last, static_unit, base - upb)
    values_phase(last, pb, static_unit, base, len(wo_last_u))

    cur = [len(wo_last_u)]

    def run_to(mark):
        while cur[0] < mark:
            advance(static_unit, base + cur[0])
            cur[0] += 1

    run_to(wo_done)
    project(G - 1)
    run_to(cur[0] + 4)
    x1 = x_buf[...].astype(_F32) + mod_scr[2] * attn_scr[...]
    h2 = _layernorm(x1) * (1.0 + mod_scr[4]) + mod_scr[3]
    y = _layernorm(h2).astype(_BF16)
    b1 = b1_buf[...].astype(_F32)
    mlp = _row_vector(b2_buf[...].astype(_F32), 0, D // _LANE)
    run_to(w1_done)
    hs = []
    tpc = _FC // _LANE
    for j in range(F // _FC):
        pre = _dot(y, w1_buf[:, :, j * _FC:(j + 1) * _FC].reshape(D, _FC))
        hs.append(_gelu_tanh(pre + _row_vector(b1, j * tpc, (j + 1) * tpc)).astype(_BF16))
        run_to(cur[0] + 3)
    hh = jnp.concatenate(hs, axis=-1)
    assert _W2_MARKS[-1] == F
    for lo, hi in zip((0,) + _W2_MARKS[:-1], _W2_MARKS):
        run_to(E - len(w2_u) + hi // _U_W2[0])
        mlp = _dot(hh[:, lo:hi], w2_buf[lo:hi, :]) + mlp
    out_buf[...] = (x1 + mod_scr[5] * mlp).astype(out_buf.dtype)
    cp_out.start()
    cp_out.wait()


def _compiler_params():
    base = dict(vmem_limit_bytes=100 * 1024 * 1024)
    try:
        return pltpu.CompilerParams(disable_bounds_checks=True, disable_semaphore_checks=True, **base)
    except TypeError:
        return pltpu.CompilerParams(**base)


def _run(A_x, A_k_cache, A_v_cache, A_wq, A_wo, B_w1, B_b1, B_w2, B_b2, c, w_mod):
    B, Sq, D = A_x.shape
    _, Hkv, Sk, Dh = A_k_cache.shape
    F = B_w1.shape[1]
    assert Sq == 1 and Hkv == _HQ and Dh == _DH and B == _SUB
    W = min(4096, max(256, Sk // 4))
    G = _HQ // _HG
    R = _HG * _DH
    GR = _KV_STRIDE * _SUB

    x2 = A_x.reshape(B, D)
    kt = jnp.swapaxes(A_k_cache, 2, 3).reshape(B * G, R // GR, GR, Sk)
    vt = jnp.swapaxes(A_v_cache, 2, 3).reshape(B * G, R // GR, GR, Sk)
    wm = w_mod.reshape(-1, _RM, w_mod.shape[1])
    wq = A_wq.reshape(-1, _RQ, A_wq.shape[1])
    wo = A_wo.reshape(-1, _RO, D)
    w1 = B_w1.reshape(-1, _R1, F)
    b1 = B_b1.reshape(F // _LANE, _LANE)
    b2 = B_b2.reshape(D // _LANE, _LANE)

    any_spec = pl.BlockSpec(memory_space=pl.ANY)
    out = pl.pallas_call(
        functools.partial(_kernel, B=B, D=D, F=F, Sk=Sk, W=W),
        in_specs=[any_spec] * 11,
        out_specs=any_spec,
        out_shape=jax.ShapeDtypeStruct((B, D), A_x.dtype),
        scratch_shapes=[
            pltpu.VMEM((2, 2, W // _CW, R // GR, GR, _CW), _BF16),
            pltpu.VMEM(wm.shape, _BF16),
            pltpu.VMEM(wq.shape, _BF16),
            pltpu.VMEM(wo.shape, _BF16),
            pltpu.VMEM(w1.shape, _BF16),
            pltpu.VMEM(B_w2.shape, _BF16),
            pltpu.VMEM(x2.shape, _BF16),
            pltpu.VMEM(c.shape, _BF16),
            pltpu.VMEM(b1.shape, _BF16),
            pltpu.VMEM(b2.shape, _BF16),
            pltpu.VMEM((B, D), A_x.dtype),
            pltpu.VMEM((6, B, D), _F32),
            pltpu.VMEM((G, B, R), _F32),
            pltpu.VMEM((B, R), _F32),
            pltpu.VMEM((B, D), _F32),
            pltpu.SemaphoreType.DMA((2 * _NS + 5,)),
        ],
        compiler_params=_compiler_params(),
    )(x2, kt, vt, wq, wo, w1, b1, B_w2, b2, c, wm)
    return out.reshape(B, Sq, D)


@jax.jit
def pallas_adaLN_cond__sliding_block_cached__mixer_channel_mlp__decode_kernel(
    A_x: jax.Array,
    A_k_cache: jax.Array,
    A_v_cache: jax.Array,
    A_wq: jax.Array,
    A_wo: jax.Array,
    B_x: jax.Array,
    B_w1: jax.Array,
    B_b1: jax.Array,
    B_w2: jax.Array,
    B_b2: jax.Array,
    c: jax.Array,
    w_mod: jax.Array,
):
    del B_x
    return _run(A_x, A_k_cache, A_v_cache, A_wq, A_wo, B_w1, B_b1, B_w2, B_b2, c, w_mod)
```

```python
import functools

import jax
import jax.numpy as jnp
from jax import lax
import jax.experimental.pallas as pl
import jax.experimental.pallas.tpu as pltpu

_F32 = jnp.float32
_BF16 = jnp.bfloat16

_HQ = 32
_DH = 192
_HG = 8
_LANE = 128
_SUB = 8

_CW = 256
_CORDER = (2, 0, 3, 1)
_KV_STRIDE = 6
_KV_N, _KV_NH = 16, 4
_DL, _DH_AHEAD, _NS = 24, 12, 24
_RM, _RQ, _RO, _R1 = 80, 80, 384, 160
_U_WM, _U_WQ, _U_WO = (8, 2, 384, 8), (8, 2, 768, 8), (6, 1, 640, 8)
_U_WO_LAST, _U_W1 = (4, 1, 640, 16), (4, 1, 1536, 8)
_WO_LAST_SPAN = 0.73
_U_W2 = (64, 16)
_W2_MARKS = (768, 1152, 1408, 1536)
_PG = 16
_GS = 2
_QW = 512
_FC = 512


def _layernorm(x, eps=1e-5):
    m = jnp.mean(x, axis=-1, keepdims=True)
    xc = x - m
    v = jnp.mean(xc * xc, axis=-1, keepdims=True)
    return xc / jnp.sqrt(v + eps)


def _gelu_tanh(x):
    return 0.5 * x * (1.0 + jnp.tanh(0.7978845608028654 * (x + 0.044715 * (x * x * x))))


def _dot(a, b):
    return jnp.dot(a, b, preferred_element_type=_F32)


def _dot_nt(a, b):
    return lax.dot_general(a, b, (((1,), (1,)), ((), ())), preferred_element_type=_F32)


def _row_vector(tiles, lo, hi):
    return jnp.concatenate([tiles[i:i + 1, :] for i in range(lo, hi)], axis=-1)


def _kernel(x_hbm, k_hbm, v_hbm, wq_hbm, wo_hbm, w1_hbm, b1_hbm, w2_hbm, b2_hbm, c_hbm, wm_hbm,
            out_hbm,
            kvbuf, wm_buf, wq_buf, wo_buf, w1_buf, w2_buf,
            x_buf, c_buf, b1_buf, b2_buf, out_buf,
            mod_scr, q_scr, o_scr, attn_scr,
            sem,
            *, B, D, F, Sk, W):
    G = _HQ // _HG
    R = _HG * _DH
    nc = W // _CW
    GR = _KV_STRIDE * _SUB
    NG = R // GR
    blk_units = [(ph, g0, c) for ph in range(_KV_STRIDE) for g0 in range(0, NG, _KV_N) for c in _CORDER]
    upb = len(blk_units)
    U = 2 * upb
    nsteps = G * B
    npc = NG // _PG
    pr = _PG * GR
    assert sorted(_CORDER) == list(range(nc))
    assert U % _NS == 0 and _DL <= min(_NS, upb) and _DH_AHEAD + _GS <= min(_NS, upb)

    def strided_units(src, dst, g_lo, g_hi, n, nh, cw, rr):
        out = []
        for r in range(0, src.shape[1], rr):
            for g0 in range(g_lo, g_hi, n):
                for c0 in range(0, src.shape[2], cw):
                    rs, cs = pl.ds(r, rr), pl.ds(c0, cw)
                    lo, hi = pl.ds(g0, n - nh), pl.ds(g0 + n - nh, nh)
                    out.append(((src.at[lo, rs, cs], dst.at[lo, rs, cs]),
                                (src.at[hi, rs, cs], dst.at[hi, rs, cs])))
        return out

    def sequential_units(src, dst, rows, hrows):
        out = []
        for r in range(0, src.shape[0], rows):
            lo, hi = pl.ds(r, rows - hrows), pl.ds(r + rows - hrows, hrows)
            out.append(((src.at[lo, :], dst.at[lo, :]), (src.at[hi, :], dst.at[hi, :])))
        return out

    gpo = wo_hbm.shape[0] // G
    wm_u = strided_units(wm_hbm, wm_buf, 0, wm_hbm.shape[0], *_U_WM)
    wq_u = strided_units(wq_hbm, wq_buf, 0, wq_hbm.shape[0], *_U_WQ)
    wo_u = strided_units(wo_hbm, wo_buf, 0, (G - 1) * gpo, *_U_WO)
    head = wm_u + wq_u + wo_u
    wo_last_u = strided_units(wo_hbm, wo_buf, (G - 1) * gpo, G * gpo, *_U_WO_LAST)
    w1_u = strided_units(w1_hbm, w1_buf, 0, w1_hbm.shape[0], *_U_W1)
    w2_u = sequential_units(w2_hbm, w2_buf, *_U_W2)
    mixed = sorted([(_WO_LAST_SPAN * (i + 1) / len(wo_last_u), 0, i) for i in range(len(wo_last_u))]
                   + [((i + 1) / len(w1_u), 1, i) for i in range(len(w1_u))])
    tail = [(wo_last_u, w1_u)[a][i] for _, a, i in mixed] + w2_u
    wo_done = 1 + max(p for p, (_, a, _) in enumerate(mixed) if a == 0)
    w1_done = len(mixed)
    P, E = len(head), len(tail)

    def split_step(step):
        if isinstance(step, int):
            g, b, slot = step // B, step % B, step % 2
        else:
            g, b, slot = lax.div(step, B), lax.rem(step, B), lax.rem(step, 2)
        return g, b, slot, b * G + g

    def kv_unit(st, u):
        isv, uu = divmod(u, upb)
        ph, g0, c = blk_units[uu]
        _, _, slot, idx = st
        src = v_hbm if isv else k_hbm
        lanes = pl.ds(Sk - W + c * _CW, _CW)
        rs = pl.ds(ph * _SUB, _SUB)
        lo, hi = pl.ds(g0, _KV_N - _KV_NH), pl.ds(g0 + _KV_N - _KV_NH, _KV_NH)
        return ((src.at[idx, lo, rs, lanes], kvbuf.at[slot, isv, c, lo, rs, :]),
                (src.at[idx, hi, rs, lanes], kvbuf.at[slot, isv, c, hi, rs, :]))

    def static_unit(pos):
        if pos < P:
            return head[pos]
        if pos < P + nsteps * U:
            return kv_unit(split_step((pos - P) // U), (pos - P) % U)
        if pos < P + nsteps * U + E:
            return tail[pos - P - nsteps * U]
        return None

    def copy(unit, pos, cls):
        s, d = unit(pos)[cls]
        return pltpu.make_async_copy(s, d, sem.at[cls * _NS + pos % _NS])

    def start(unit, pos, cls):
        if unit(pos) is not None:
            copy(unit, pos, cls).start(priority=1 - cls)

    def advance(unit, pos, skip_high=False):
        copy(unit, pos, 0).wait()
        copy(unit, pos, 1).wait()
        if not skip_high:
            start(unit, pos + _DH_AHEAD, 1)
        start(unit, pos + _DL, 0)

    def phase(unit, pos0, nslots, nitems, item):
        nbursts = nitems // _GS
        at = {(i * (nslots - _GS)) // nbursts: i for i in range(nbursts)}
        assert len(at) == nbursts
        early = set()
        for u in range(nslots):
            advance(unit, pos0 + u, skip_high=u in early)
            if u in at:
                for j in range(_GS):
                    item(at[u] * _GS + j)
                    if u + 1 + j not in early:
                        start(unit, pos0 + u + 1 + j + _DH_AHEAD, 1)
                        early.add(u + 1 + j)

    small = [pltpu.make_async_copy(s, d, sem.at[2 * _NS + i]) for i, (s, d) in enumerate(
        [(c_hbm, c_buf), (x_hbm, x_buf), (b1_hbm, b1_buf), (b2_hbm, b2_buf)])]
    cp_out = pltpu.make_async_copy(out_buf, out_hbm, sem.at[2 * _NS + len(small)])

    for p in range(_DL):
        start(static_unit, p, 0)
        if p < _DH_AHEAD:
            start(static_unit, p, 1)
    for cp in small:
        cp.start()

    def wait_small():
        for cp in small:
            cp.wait()
        attn_scr[...] = jnp.zeros_like(attn_scr)

    def mod_piece(j):
        c = c_buf[...].astype(_F32)
        silu_c = (c * jax.nn.sigmoid(c)).astype(_BF16)
        mod_scr[j] = _dot(silu_c, wm_buf[:, :, j * D:(j + 1) * D].reshape(D, D))

    def h_piece():
        mod_scr[0] = _layernorm(x_buf[...].astype(_F32)) * (1.0 + mod_scr[1]) + mod_scr[0]

    def q_piece(j):
        q = _dot(mod_scr[0].astype(_BF16), wq_buf[:, :, j * _QW:(j + 1) * _QW].reshape(D, _QW))
        g, o = divmod(j * _QW, R)
        q_scr[g, :, o:o + _QW] = q.astype(_BF16).astype(_F32)

    after = {len(wm_u) - 2: wait_small, len(wm_u) + 24: h_piece}
    for j in range(6):
        after[len(wm_u) - 1 + 4 * j] = functools.partial(mod_piece, j)
    for j in range(_HQ * _DH // _QW):
        after[len(wm_u) + len(wq_u) - 1 + 3 * j] = functools.partial(q_piece, j)
    assert len(after) == 8 + _HQ * _DH // _QW and max(after) < P + upb
    for p in range(P + upb):
        advance(static_unit, p)
        if p in after:
            after[p]()

    row = lax.broadcasted_iota(jnp.int32, (_HG, R), 0)
    col = lax.broadcasted_iota(jnp.int32, (_HG, R), 1)
    diag = (col >= row * _DH) & (col < (row + 1) * _DH)
    scale = float(_DH) ** -0.5

    def kv_piece(slot, isv, c, r):
        return kvbuf[slot, isv, c, r * _PG:(r + 1) * _PG].reshape(pr, _CW)

    def scores_phase(st, unit, pos0):
        g, b, slot, _ = st
        qrow = q_scr[g, pl.ds(b, 1), :]
        qbd = jnp.where(diag, jnp.broadcast_to(qrow, (_HG, R)), 0.0).astype(_BF16)
        parts = [None] * nc

        def item(i):
            r, c = divmod(i, nc)
            t = _dot(qbd[:, r * pr:(r + 1) * pr], kv_piece(slot, 0, c, r))
            parts[c] = t if r == 0 else t + parts[c]
        phase(unit, pos0, upb, npc * nc, item)
        s = jnp.concatenate(parts, axis=-1) * scale
        p = jnp.exp(s - jnp.max(s, axis=-1, keepdims=True))
        return (p / jnp.sum(p, axis=-1, keepdims=True)).astype(_BF16)

    def values_phase(st, pb, unit, pos0, nslots):
        _, b, slot, _ = st
        parts = [None] * npc

        def item(i):
            r, c = divmod(i, nc)
            t = _dot_nt(pb[:, c * _CW:(c + 1) * _CW], kv_piece(slot, 1, c, r))
            parts[r] = t if c == 0 else t + parts[r]
        phase(unit, pos0, nslots, npc * nc, item)
        o = jnp.where(diag, jnp.concatenate(parts, axis=-1), 0.0)
        o_scr[pl.ds(b, 1), :] = jnp.sum(o, axis=0, keepdims=True)

    def project(g):
        attn_scr[...] += _dot(o_scr[...].astype(_BF16), wo_buf[pl.ds(g * gpo, gpo)].reshape(R, D))

    def step_body(step, carry):
        st, st_next = split_step(step), split_step(step + 1)

        def unit(pos):
            u = pos - P
            return kv_unit(st, u) if u < U else kv_unit(st_next, u - U)
        pb = scores_phase(st, unit, P + upb)
        values_phase(st, pb, unit, P + U, upb)

        @pl.when(st[1] == B - 1)
        def _():
            project(st[0])
        return carry

    lax.fori_loop(0, nsteps - 1, step_body, 0)
    last = split_step(nsteps - 1)
    base = P + nsteps * U
    pb = scores_phase(last, static_unit, base - upb)
    values_phase(last, pb, static_unit, base, len(wo_last_u))

    cur = [len(wo_last_u)]

    def run_to(mark):
        while cur[0] < mark:
            advance(static_unit, base + cur[0])
            cur[0] += 1

    run_to(wo_done)
    project(G - 1)
    run_to(cur[0] + 4)
    x1 = x_buf[...].astype(_F32) + mod_scr[2] * attn_scr[...]
    h2 = _layernorm(x1) * (1.0 + mod_scr[4]) + mod_scr[3]
    y = _layernorm(h2).astype(_BF16)
    b1 = b1_buf[...].astype(_F32)
    mlp = _row_vector(b2_buf[...].astype(_F32), 0, D // _LANE)
    run_to(w1_done)
    hs = []
    tpc = _FC // _LANE
    for j in range(F // _FC):
        pre = _dot(y, w1_buf[:, :, j * _FC:(j + 1) * _FC].reshape(D, _FC))
        hs.append(_gelu_tanh(pre + _row_vector(b1, j * tpc, (j + 1) * tpc)).astype(_BF16))
        run_to(cur[0] + 3)
    hh = jnp.concatenate(hs, axis=-1)
    assert _W2_MARKS[-1] == F
    for lo, hi in zip((0,) + _W2_MARKS[:-1], _W2_MARKS):
        run_to(E - len(w2_u) + hi // _U_W2[0])
        mlp = _dot(hh[:, lo:hi], w2_buf[lo:hi, :]) + mlp
    out_buf[...] = (x1 + mod_scr[5] * mlp).astype(out_buf.dtype)
    cp_out.start()
    cp_out.wait()


def _compiler_params():
    base = dict(vmem_limit_bytes=100 * 1024 * 1024)
    try:
        return pltpu.CompilerParams(disable_bounds_checks=True, disable_semaphore_checks=True, **base)
    except TypeError:
        return pltpu.CompilerParams(**base)


def _run(A_x, A_k_cache, A_v_cache, A_wq, A_wo, B_w1, B_b1, B_w2, B_b2, c, w_mod):
    B, Sq, D = A_x.shape
    _, Hkv, Sk, Dh = A_k_cache.shape
    F = B_w1.shape[1]
    assert Sq == 1 and Hkv == _HQ and Dh == _DH and B == _SUB
    W = min(4096, max(256, Sk // 4))
    G = _HQ // _HG
    R = _HG * _DH
    GR = _KV_STRIDE * _SUB

    x2 = A_x.reshape(B, D)
    kt = jnp.swapaxes(A_k_cache, 2, 3).reshape(B * G, R // GR, GR, Sk)
    vt = jnp.swapaxes(A_v_cache, 2, 3).reshape(B * G, R // GR, GR, Sk)
    wm = w_mod.reshape(-1, _RM, w_mod.shape[1])
    wq = A_wq.reshape(-1, _RQ, A_wq.shape[1])
    wo = A_wo.reshape(-1, _RO, D)
    w1 = B_w1.reshape(-1, _R1, F)
    b1 = B_b1.reshape(F // _LANE, _LANE)
    b2 = B_b2.reshape(D // _LANE, _LANE)

    any_spec = pl.BlockSpec(memory_space=pl.ANY)
    out = pl.pallas_call(
        functools.partial(_kernel, B=B, D=D, F=F, Sk=Sk, W=W),
        in_specs=[any_spec] * 11,
        out_specs=any_spec,
        out_shape=jax.ShapeDtypeStruct((B, D), A_x.dtype),
        scratch_shapes=[
            pltpu.VMEM((2, 2, W // _CW, R // GR, GR, _CW), _BF16),
            pltpu.VMEM(wm.shape, _BF16),
            pltpu.VMEM(wq.shape, _BF16),
            pltpu.VMEM(wo.shape, _BF16),
            pltpu.VMEM(w1.shape, _BF16),
            pltpu.VMEM(B_w2.shape, _BF16),
            pltpu.VMEM(x2.shape, _BF16),
            pltpu.VMEM(c.shape, _BF16),
            pltpu.VMEM(b1.shape, _BF16),
            pltpu.VMEM(b2.shape, _BF16),
            pltpu.VMEM((B, D), A_x.dtype),
            pltpu.VMEM((6, B, D), _F32),
            pltpu.VMEM((G, B, R), _F32),
            pltpu.VMEM((B, R), _F32),
            pltpu.VMEM((B, D), _F32),
            pltpu.SemaphoreType.DMA((2 * _NS + 5,)),
        ],
        compiler_params=_compiler_params(),
    )(x2, kt, vt, wq, wo, w1, b1, B_w2, b2, c, wm)
    return out.reshape(B, Sq, D)


@jax.jit
def pallas_adaLN_cond__sliding_block_cached__mixer_channel_mlp__decode_kernel(
    A_x: jax.Array,
    A_k_cache: jax.Array,
    A_v_cache: jax.Array,
    A_wq: jax.Array,
    A_wo: jax.Array,
    B_x: jax.Array,
    B_w1: jax.Array,
    B_b1: jax.Array,
    B_w2: jax.Array,
    B_b2: jax.Array,
    c: jax.Array,
    w_mod: jax.Array,
):
    del B_x
    return _run(A_x, A_k_cache, A_v_cache, A_wq, A_wo, B_w1, B_b1, B_w2, B_b2, c, w_mod)
```
